```python
import jax
import jax.numpy as jnp

def _softmax(x, axis=-1):
    return jax.nn.softmax(x, axis=axis)
def _gelu(x):
    return jax.nn.gelu(x, approximate=True)
def _silu(x):
    return jax.nn.silu(x)
def _sigmoid(x):
    return jax.nn.sigmoid(x)
def _layernorm(x, axis=-1, eps=1e-5):
    m = jnp.mean(x, axis=axis, keepdims=True)
    v = jnp.var(x, axis=axis, keepdims=True)
    return (x - m) / jnp.sqrt(v + eps)
def _scatter_add(tgt, idx, src, axis=0):
    return tgt.at[idx].add(src)
def _segment_sum(src, seg, n):
    return jax.ops.segment_sum(src, seg, n)
class _Rng:
    def __init__(self, key):
        self._k = key
    def _next(self):
        self._k, sub = jax.random.split(self._k)
        return sub
    def normal(self, shape):
        return jax.random.normal(self._next(), shape, dtype=jnp.bfloat16)
    def randint(self, lo, hi, shape):
        return jax.random.randint(self._next(), shape, lo, hi, dtype=jnp.int32)
    def uniform(self, shape, lo=0.0, hi=1.0):
        return jax.random.uniform(self._next(), shape, jnp.bfloat16, lo, hi)
    def permutation(self, n):
        return jax.random.permutation(self._next(), n)


kernel_name = 'sequential_preLN__mha_block_cached__moe_arch_mod__decode'

def setup_inputs():
    _rng = _Rng(jax.random.key(int.from_bytes(__import__("os").urandom(4), "little")))
    _w = (lambda a: (lambda t: t.astype(jnp.bfloat16) if jnp.issubdtype(t.dtype, jnp.floating) else t)(jnp.asarray(a)))
    def _A_setup():
        B, Sq, D = 4, 1, 640
        H, Sk, Dh = 32, 8192, 192
        return {
            "x": _w((lambda *s: _rng.normal(s) * 0.05)(B, Sq, D)),
            "k_cache": _w((lambda *s: _rng.normal(s) * 0.05)(B, H, Sk, Dh)),
            "v_cache": _w((lambda *s: _rng.normal(s) * 0.05)(B, H, Sk, Dh)),
            "wq": _w((lambda *s: _rng.normal(s) * 0.05)(D, H * Dh) * (D ** -0.5)),
            "wo": _w((lambda *s: _rng.normal(s) * 0.05)(H * Dh, D) * ((H * Dh) ** -0.5)),
        }
    _A_in = _A_setup()

    def _B_setup():
        B, S, D, F, C = 4, 1, 640, 1536, 1
        return {
            "x": _w((lambda *s: _rng.normal(s) * 0.05)(B, S, D)),
            "w_r": _w((lambda *s: _rng.normal(s) * 0.05)(D)),
            "w_gate": _w((lambda *s: _rng.normal(s) * 0.05)(D, F)),
            "w_up": _w((lambda *s: _rng.normal(s) * 0.05)(D, F)),
            "w_down": _w((lambda *s: _rng.normal(s) * 0.05)(F, D)),
        }
    _B_in = _B_setup()

    return {
        "A_x": _A_in["x"],
        "A_k_cache": _A_in["k_cache"],
        "A_v_cache": _A_in["v_cache"],
        "A_wq": _A_in["wq"],
        "A_wo": _A_in["wo"],
        "B_x": _B_in["x"],
        "B_w_r": _B_in["w_r"],
        "B_w_gate": _B_in["w_gate"],
        "B_w_up": _B_in["w_up"],
        "B_w_down": _B_in["w_down"],
    }

def reference(A_x, A_k_cache, A_v_cache, A_wq, A_wo, B_x, B_w_r, B_w_gate, B_w_up, B_w_down):
    def _A_ref(x, k_cache, v_cache, wq, wo):
        B, Sq, D = x.shape
        H, Dh = 32, 192
        q = (lambda x, *d: x.transpose(*d))((x @ wq).reshape(B, Sq, H, Dh), 0, 2, 1, 3)
        scores = jnp.einsum("bhqd,bhkd->bhqk", q, k_cache) * (Dh ** -0.5)
        p = _softmax(scores, axis=-1)
        o = jnp.einsum("bhqk,bhkd->bhqd", p, v_cache)
        return (lambda x, *d: x.transpose(*d))(o, 0, 2, 1, 3).reshape(B, Sq, H * Dh) @ wo

    def _B_ref(x, w_r, w_gate, w_up, w_down):
        B, S, D = x.shape
        C = 1
        r = x @ w_r
        idx = jnp.argsort(-r, axis=-1)[:, :C]
        idx_e = jnp.repeat(idx.reshape(B, C, 1), D, axis=2)
        x_sel = jnp.take_along_axis(x, idx_e, axis=1)
        g = _silu(x_sel @ w_gate)
        u = x_sel @ w_up
        y = (g * u) @ w_down
        r_sel = _sigmoid(jnp.take_along_axis(r, idx, axis=1))
        y = y * r_sel.reshape(B, C, 1)
        b_off = (jnp.arange(B) * S).reshape(B, 1)
        flat_idx = (idx + b_off).reshape(B * C)
        zero = (x * 0.0).reshape(B * S, D)
        upd = _scatter_add(zero, flat_idx, y.reshape(B * C, D), axis=0)
        return x + upd.reshape(B, S, D)

    x = A_x
    h = x + _A_ref(_layernorm(x, axis=-1), A_k_cache, A_v_cache, A_wq, A_wo)
    h2 = h + _B_ref(_layernorm(h, axis=-1), B_w_r, B_w_gate, B_w_up, B_w_down)
    return h2
```

```python
import functools

import jax
import jax.numpy as jnp
import jax.experimental.pallas as pl
import jax.experimental.pallas.tpu as pltpu

_EPS = 1e-5
_NB = 2
_WIN = 512
_BLK = 64
_GC = 1024
_PACE = 2
_K_PAD = 336
_V_PAD = 544
_RING = 8
_FW = 256


def _layernorm(x):
    m = jnp.mean(x, axis=-1, keepdims=True)
    d = x - m
    v = jnp.mean(d * d, axis=-1, keepdims=True)
    return d / jnp.sqrt(v + _EPS)


def _dot(a, b):
    return jnp.dot(a, b, preferred_element_type=jnp.float32)


def _dot_nt(a, b):
    return jax.lax.dot_general(
        a, b, (((1,), (1,)), ((), ())), preferred_element_type=jnp.float32
    )


def _wait_all(buf, sem):
    pltpu.make_async_copy(buf, buf, sem).wait()


def _ds(start, size):
    return pl.ds(start if isinstance(start, int) else pl.multiple_of(start, size), size)


def _loop(lo, hi, fn):
    jax.lax.fori_loop(lo, hi, lambda i, carry: fn(i), None)


def _body(
    x_hbm, kt_hbm, vt_hbm, wq_hbm, wo_hbm, wr_hbm, wg_hbm, wu_hbm, wd_hbm,
    out_ref,
    kbuf, vbuf, wqbuf, wobuf, wgbuf, wubuf, wdbuf, xbuf, wrbuf,
    q_scr, o_scr, s_scr, p_scr, l_scr,
    ksem, vsem, wqsem, wosem, msem, gsem, usem, dsem,
    *, B, H, Dh, Sk, D, F,
):
    HD = H * Dh
    rows_total = B * HD
    last = rows_total // _WIN
    n_blk = _WIN // _BLK
    n_cc = Sk // _GC
    n_rt = _BLK // 8
    lead = n_rt * n_cc - 2 * n_cc * _PACE
    NF = F // _FW
    scale = Dh ** -0.5
    f32, bf16 = jnp.float32, jnp.bfloat16

    def piece(hbm, buf, sem, pad, p, rt, cc, blk, n, queue):
        row = p * _WIN - pad + rt * 8
        cols = _ds(cc * _GC, _GC)
        slot = p % _NB
        pltpu.make_async_copy(
            hbm.at[pl.ds((row >> 6) + blk, n), _ds(row & (_BLK - 1), 8), cols],
            buf.at[slot, pl.ds(blk, n), _ds(rt * 8, 8), cols],
            sem.at[slot],
        ).start(priority=queue)

    k_piece = functools.partial(piece, kt_hbm, kbuf, ksem, _K_PAD)
    v_piece = functools.partial(piece, vt_hbm, vbuf, vsem, _V_PAD)

    def blocks(pad, p, rt):
        out = []
        for s in range(0, n_blk, 2):
            rows = [p * _WIN - pad + (s + i) * _BLK + rt * 8 for i in range(2)]
            inside = [s + i for i in range(2) if 0 <= rows[i] < rows_total]
            if inside:
                out.append((inside[0], len(inside)))
        return out

    def issue_visits(p, first, count):
        def visit(i):
            rt, cc = i >> 3, i & (n_cc - 1)
            for s in range(0, n_blk, 2):
                k_piece(p, rt, cc, s, 2, 0)
                v_piece(p, rt, cc, s, 2, 1)

        _loop(first, first + count, visit)

    def issue_edge(p, rt, first, end):
        ks = [(k_piece, b) for b in blocks(_K_PAD, p, rt)]
        vs = [(v_piece, b) for b in blocks(_V_PAD, p, rt)]
        todo = [c for i in range(n_blk // 2) for c in ks[i:i + 1] + vs[i:i + 1]]

        def two_visits(i):
            for j in range(2):
                for k, (fn, (blk, n)) in enumerate(todo):
                    fn(p, i >> 2, (2 * i + j) & (n_cc - 1), blk, n, (k + j * len(todo)) % 2)

        if todo:
            _loop(first, end, two_visits)

    def wait_window(buf, sem, pad, p):
        lo, hi = max(0, pad - p * _WIN), min(_WIN, rows_total + pad - p * _WIN)
        full, rest = divmod(hi - lo, _BLK)
        if full:
            _wait_all(buf.at[0, pl.ds(0, full)], sem.at[p % _NB])
        if rest:
            _wait_all(buf.at[0, 0, pl.ds(0, rest)], sem.at[p % _NB])

    def issue_wq():
        per_row = HD // _GC
        n = D // 8 * per_row

        def visit(i, streams):
            for s in range(streams):
                g = s * 64 + i
                where = (_ds(g // per_row * 8, 8), _ds(g % per_row * _GC, _GC))
                pltpu.make_async_copy(
                    wq_hbm.at[where], wqbuf.at[where], wqsem.at[0]
                ).start(priority=s % 2)

        _loop(0, n % 64, lambda i: visit(i, n // 64 + 1))
        _loop(n % 64, 64, lambda i: visit(i, n // 64))

    wo_rows = HD // 8

    def issue_wo(i):
        for s in range(8):
            rows = pl.ds(pl.multiple_of(s * wo_rows + i * 24, 8), 24)
            pltpu.make_async_copy(wo_hbm.at[rows], wobuf.at[rows], wosem.at[0]).start(
                priority=s % 2
            )

    def issue_gate_up(f):
        cols = _ds(f * _FW, _FW)
        for r in range(0, D, 64):
            rows = pl.ds(r, 64)
            pltpu.make_async_copy(
                wg_hbm.at[rows, cols], wgbuf.at[f, rows, :], gsem.at[f]
            ).start(priority=0)
            pltpu.make_async_copy(
                wu_hbm.at[rows, cols], wubuf.at[f, rows, :], usem.at[f]
            ).start(priority=1)

    def issue_down(f):
        for i, r in enumerate(range(0, _FW, 32)):
            pltpu.make_async_copy(
                wd_hbm.at[_ds(f * _FW + r, 32), :], wdbuf.at[f, pl.ds(r, 32), :], dsem.at[f]
            ).start(priority=i % 2)

    ring_row = jax.lax.broadcasted_iota(jnp.int32, (_RING, _GC), 0)
    lane = jax.lax.broadcasted_iota(jnp.int32, (_RING, _GC), 1)

    def owned(first_row, width):
        span = _RING * Dh
        r = lane[:, :width] + (first_row + span) % span
        r = jnp.where(r >= span, r - span, r)
        lo = ring_row[:, :width] * Dh
        return (r >= lo) & (r < lo + Dh)

    def score_chunk(p, cc, lo=0, hi=_WIN):
        q = q_scr[:, pl.ds(pl.multiple_of(p * _WIN + lo, 128), hi - lo)].astype(bf16)
        cols = _ds(cc * _GC, _GC)
        k = kbuf[p % _NB, pl.ds(lo // _BLK, (hi - lo) // _BLK), :, cols]
        s_scr[:, cols] += _dot(q, k.reshape(hi - lo, _GC))

    def softmax(p):
        end = (p + 1) * _WIN - _K_PAD
        done_hi = jnp.minimum(end, rows_total) // Dh
        done_lo = jnp.maximum(end - _WIN, 0) // Dh
        age = (ring_row[:, :1] - done_lo % _RING + _RING) % _RING
        done = age < done_hi - done_lo
        raw = s_scr[...]
        s = raw * scale
        e = jnp.exp(s - jnp.max(s, axis=-1, keepdims=True))
        p_scr[...] = jnp.where(done, e, p_scr[...])
        l_scr[...] = jnp.where(done, jnp.sum(e, axis=-1, keepdims=True), l_scr[...])
        s_scr[...] = jnp.where(done, 0.0, raw)

    def value_chunk(p, cc, hi=_WIN):
        cols = _ds(cc * _GC, _GC)
        v = vbuf[p % _NB, pl.ds(0, hi // _BLK), :, cols]
        return _dot_nt(p_scr[:, cols].astype(bf16), v.reshape(hi, _GC))

    def store_values(p, pv):
        width = pv.shape[1]
        o = jnp.where(owned(p * _WIN - _V_PAD, width), pv / l_scr[...], 0.0)
        o_scr[:, pl.ds(pl.multiple_of(p * _WIN, _WIN), width)] = o

    def attend(p, issue_a, issue_b, k_hi=_WIN):
        def score(i):
            issue_a(i)
            score_chunk(p, i, 0, k_hi)

        def value(i, acc):
            issue_b(i)
            return acc + value_chunk(p, i)

        _loop(0, n_cc, score)
        softmax(p)
        zero = jnp.zeros((_RING, _WIN), f32)
        store_values(p, jax.lax.fori_loop(0, n_cc, value, zero))

    x_cp = pltpu.make_async_copy(x_hbm, xbuf, msem.at[0])
    wr_cp = pltpu.make_async_copy(wr_hbm, wrbuf, msem.at[1])
    issue_wq()
    x_cp.start()
    wr_cp.start(priority=1)
    cut = _K_PAD % _BLK // 8
    issue_edge(0, 0, 0, 4 * cut)
    issue_edge(0, cut, 4 * cut, 4 * n_rt)

    k_lo = _K_PAD // 128 * 128
    for buf, slot, lo, hi in ((kbuf, 0, k_lo, _K_PAD), (vbuf, 1 % _NB, 0, _V_PAD - _WIN)):
        for r in range(lo, hi, 16):
            buf[slot, r // _BLK, pl.ds(r % _BLK, 16), :] = jnp.zeros((16, Sk), buf.dtype)
    s_scr[...] = jnp.zeros_like(s_scr)
    p_scr[...] = jnp.zeros_like(p_scr)
    l_scr[...] = jnp.ones_like(l_scr)
    q_scr[:, pl.ds(0, _WIN)] = jnp.zeros((_RING, _WIN), f32)
    q_scr[:, pl.ds(rows_total, _WIN)] = jnp.zeros((_RING, _WIN), f32)

    x_cp.wait()
    x4 = xbuf[...].astype(f32)
    x = jnp.concatenate([x4, x4], axis=0)
    xn = _layernorm(x).astype(bf16)
    _wait_all(wqbuf, wqsem.at[0])
    n_q = HD // _GC
    for c in range(n_q):
        if c < n_rt // 2:
            issue_edge(1, c, 4 * c, 4 * c + 4)
        else:
            issue_visits(1, c * n_cc, n_cc)
        q = _dot(xn, wqbuf[:, pl.ds(c * _GC, _GC)])
        mine = owned(c * _GC, _GC)
        for b in range(B):
            q_scr[:, pl.ds(_K_PAD + b * HD + c * _GC, _GC)] = jnp.where(mine, q[b:b + 1], 0.0)
    wait_window(kbuf, ksem, _K_PAD, 0)
    per = (n_rt - n_q)

    def first_scores(i):
        issue_visits(1, n_q * n_cc + i * per, per)
        score_chunk(0, i, k_lo)

    _loop(0, n_cc, first_scores)
    softmax(0)
    issue_visits(2, 0, lead)

    def window(p):
        slot = p % _NB
        _wait_all(kbuf.at[0], ksem.at[slot])
        pl.when(p == 1)(lambda: wait_window(vbuf, vsem, _V_PAD, 1))
        pl.when(p > 1)(lambda: _wait_all(vbuf.at[0], vsem.at[slot]))
        attend(
            p,
            lambda i: issue_visits(p + 1, lead + i * _PACE, _PACE),
            lambda i: issue_visits(p + 1, lead + (n_cc + i) * _PACE, _PACE),
        )
        pl.when(p + 2 < last)(lambda: issue_visits(p + 2, 0, lead))

    _loop(1, last - 1, window)

    def paced(i):
        return lead // 2 + i * _PACE // 2

    issue_edge(last, 0, 0, 4 * cut)
    issue_edge(last, cut, 4 * cut, paced(0))
    wait_window(kbuf, ksem, _K_PAD, last - 1)
    wait_window(vbuf, vsem, _V_PAD, last - 1)
    attend(
        last - 1,
        lambda i: issue_edge(last, cut, paced(i), paced(i + 1)),
        lambda i: issue_edge(last, cut, paced(n_cc + i), paced(n_cc + i + 1)),
    )
    issue_edge(last + 1, 0, 0, 4 * (_V_PAD - _WIN) // 8)
    wo_lead = wo_rows // 24 - 2 * n_cc
    _loop(0, wo_lead, issue_wo)
    wait_window(kbuf, ksem, _K_PAD, last)
    wait_window(vbuf, vsem, _V_PAD, last)
    attend(
        last,
        lambda i: issue_wo(wo_lead + i),
        lambda i: issue_wo(wo_lead + n_cc + i),
        -(-_K_PAD // 128) * 128,
    )
    issue_gate_up(0)
    wait_window(vbuf, vsem, _V_PAD, last + 1)
    store_values(last + 1, sum(value_chunk(last + 1, cc, 128) for cc in range(n_cc)))
    o = jnp.concatenate(
        [o_scr[:, pl.ds(_V_PAD + b * HD, HD)] for b in range(B)], axis=0
    ).astype(bf16)
    _loop(1, NF, issue_gate_up)
    _wait_all(wobuf, wosem.at[0])
    attn = jnp.zeros((B * _RING, D), f32)
    step = HD // NF
    for f in range(NF):
        issue_down(f)
        attn = attn + _dot(o[:, f * step:(f + 1) * step], wobuf[pl.ds(f * step, step), :])
    attn = jnp.sum(attn.reshape(B, _RING, D), axis=1)
    h = x + jnp.concatenate([attn, attn], axis=0)
    hn = _layernorm(h)
    hb = hn.astype(bf16)
    wr_cp.wait()
    r = jnp.sum(hn * wrbuf[...].astype(f32).reshape(1, D), axis=-1, keepdims=True)
    acts = []
    for f in range(NF):
        _wait_all(wgbuf.at[f], gsem.at[f])
        _wait_all(wubuf.at[f], usem.at[f])
        gate = _dot(hb, wgbuf[f])
        up = _dot(hb, wubuf[f])
        acts.append((gate * jax.nn.sigmoid(gate) * up).astype(bf16))
    y = jnp.zeros((2 * B, D), f32)
    for f in range(NF):
        _wait_all(wdbuf.at[f], dsem.at[f])
        y = y + _dot(acts[f], wdbuf[f])
    y = y * jax.nn.sigmoid(r)
    out = h + (hn + (hn * 0.0 + y))
    out_ref[...] = out[:B].astype(out_ref.dtype)


@jax.jit
def pallas_sequential_preLN__mha_block_cached__moe_arch_mod__decode_kernel(
    A_x: jax.Array,
    A_k_cache: jax.Array,
    A_v_cache: jax.Array,
    A_wq: jax.Array,
    A_wo: jax.Array,
    B_x: jax.Array,
    B_w_r: jax.Array,
    B_w_gate: jax.Array,
    B_w_up: jax.Array,
    B_w_down: jax.Array,
):
    del B_x
    B, Sq, D = A_x.shape
    _, H, Sk, Dh = A_k_cache.shape
    F = B_w_gate.shape[1]
    HD = H * Dh
    assert (Sq, B, Sk) == (1, 4, 8 * _GC) and H % _RING == 0 and HD % _GC == 0
    assert _V_PAD - _K_PAD >= Dh and F % _FW == 0 and D % 64 == 0
    dt = A_k_cache.dtype
    f32 = jnp.float32

    kt = jnp.swapaxes(A_k_cache, 2, 3).reshape(B * HD // _BLK, _BLK, Sk)
    vt = jnp.swapaxes(A_v_cache, 2, 3).reshape(B * HD // _BLK, _BLK, Sk)

    out = pl.pallas_call(
        functools.partial(_body, B=B, H=H, Dh=Dh, Sk=Sk, D=D, F=F),
        in_specs=[pl.BlockSpec(memory_space=pl.ANY)] * 9,
        out_specs=pl.BlockSpec(memory_space=pltpu.VMEM),
        out_shape=jax.ShapeDtypeStruct((B, D), A_x.dtype),
        scratch_shapes=[
            pltpu.VMEM((_NB, _WIN // _BLK, _BLK, Sk), dt),
            pltpu.VMEM((_NB, _WIN // _BLK, _BLK, Sk), dt),
            pltpu.VMEM((D, HD), dt),
            pltpu.VMEM((HD, D), dt),
            pltpu.VMEM((F // _FW, D, _FW), dt),
            pltpu.VMEM((F // _FW, D, _FW), dt),
            pltpu.VMEM((F // _FW, _FW, D), dt),
            pltpu.VMEM((B, D), dt),
            pltpu.VMEM((D,), dt),
            pltpu.VMEM((_RING, B * HD + _WIN), f32),
            pltpu.VMEM((_RING, B * HD + 2 * _WIN), f32),
            pltpu.VMEM((_RING, Sk), f32),
            pltpu.VMEM((_RING, Sk), f32),
            pltpu.VMEM((_RING, 1), f32),
            pltpu.SemaphoreType.DMA((_NB,)),
            pltpu.SemaphoreType.DMA((_NB,)),
            pltpu.SemaphoreType.DMA((1,)),
            pltpu.SemaphoreType.DMA((1,)),
            pltpu.SemaphoreType.DMA((2,)),
            pltpu.SemaphoreType.DMA((F // _FW,)),
            pltpu.SemaphoreType.DMA((F // _FW,)),
            pltpu.SemaphoreType.DMA((F // _FW,)),
        ],
        compiler_params=pltpu.CompilerParams(vmem_limit_bytes=96 * 1024 * 1024),
    )(A_x.reshape(B, D), kt, vt, A_wq, A_wo, B_w_r, B_w_gate, B_w_up, B_w_down)
    return out.reshape(B, Sq, D)
```

```python
import functools

import jax
import jax.numpy as jnp
import jax.experimental.pallas as pl
import jax.experimental.pallas.tpu as pltpu

_EPS = 1e-5
_NOCHECK = True
_NB = 3
_WIN = 512
_QTR = 128
_GC = 1024
_VISITS = 64
_STEPS = 16
_LEAD = 16
_PACE = (3, 2, 2, 2, 4)
_K_PAD = 336
_V_PAD = 544
_RING = 8
_RUNS = (16, 8, 8, 16, 8, 4, 4)
_EARLY = 4
_DOWN = 0
_SLAB = 32
_PARTS = 6


def _layernorm(x):
    m = jnp.mean(x, axis=-1, keepdims=True)
    d = x - m
    v = jnp.mean(d * d, axis=-1, keepdims=True)
    return d / jnp.sqrt(v + _EPS)


def _dot(a, b):
    return jnp.dot(a, b, preferred_element_type=jnp.float32)


def _dot_nt(a, b):
    return jax.lax.dot_general(
        a, b, (((1,), (1,)), ((), ())), preferred_element_type=jnp.float32
    )


def _wait_all(buf, sem):
    pltpu.make_async_copy(buf, buf, sem).wait()


def _ds(start, size):
    return pl.ds(start if isinstance(start, int) else pl.multiple_of(start, size), size)


def _loop(lo, hi, fn):
    jax.lax.fori_loop(lo, hi, lambda i, carry: fn(i), None)


def _body(
    x_hbm, kt_hbm, vt_hbm, wq_hbm, wo_hbm, wr_hbm, wg_hbm, wu_hbm, wd_hbm,
    out_ref,
    kbuf, vbuf, vend, wqbuf, wobuf, wgbuf, wubuf, wdbuf, xbuf, wrbuf,
    x_scr, n_scr, t_scr, q_scr, o_scr, ob_scr, s_scr, p_scr, l_scr, pv_scr, a_scr, g_scr, y_scr,
    ksem, vsem, dsem, sem,
    *, B, H, Dh, Sk, D, F,
):
    HD = H * Dh
    last = B * HD // _WIN
    k_first = _WIN - _K_PAD
    v_end = _V_PAD - _WIN
    half = _STEPS // 2
    scale = Dh ** -0.5
    f32, bf16 = jnp.float32, jnp.bfloat16
    X, WR, WQ, VE, WO, GU0, GU1 = (sem.at[i] for i in range(7))

    def copy(src, dst, dma_sem, queue):
        pltpu.make_async_copy(src, dst, dma_sem).start(priority=queue)

    def cache_piece(hbm, buf, dma_sem, row, buf_row):
        def piece(g, queue):
            r, cols = (g >> 2) * 8, _ds((g & 3) * 2 * _GC, 2 * _GC)
            src, dst = row + r, buf_row + r
            copy(
                hbm.at[src >> 7, _ds(src & (_QTR - 1), 8), cols],
                buf.at[dst >> 7, _ds(dst & (_QTR - 1), 8), cols],
                dma_sem,
                queue,
            )

        return piece

    def wq_piece(g, queue):
        row = g * 171 >> 9
        where = (_ds(row * 8, 8), _ds((g - 3 * row) * 2 * _GC, 2 * _GC))
        copy(wq_hbm.at[where], wqbuf.at[where], WQ, queue)

    def row_piece(hbm, buf, dma_sem, rows, cols=slice(None)):
        def piece(g, queue):
            where = (_ds(g * rows, rows), cols)
            copy(hbm.at[where], buf.at[where], dma_sem, queue)

        return piece

    def down_piece(first):
        def piece(g, queue):
            rows = _ds((first + g) * _SLAB, _SLAB)
            copy(wd_hbm.at[rows], wdbuf.at[rows], dsem.at[(first + g) >> 3], queue)

        return piece

    end_slot = last % _NB
    units = F // _PARTS
    early, late = pl.ds(0, _EARLY * units), pl.ds(_EARLY * units, F - _EARLY * units)
    k_end = cache_piece(kt_hbm, kbuf.at[end_slot], ksem.at[end_slot], B * HD - _K_PAD, 0)
    v_last = cache_piece(vt_hbm, vbuf.at[end_slot], vsem.at[end_slot], B * HD - _V_PAD, 0)
    head = (
        ([wq_piece], D // 8 * HD // (2 * _GC), _RUNS[0]),
        ([cache_piece(kt_hbm, kbuf.at[0], ksem.at[0], 0, _K_PAD)], k_first // 2, _RUNS[1]),
    )
    tail = (
        ([k_end], _K_PAD // 2, _RUNS[2]),
        ([v_last], _WIN // 2, _RUNS[3]),
        ([cache_piece(vt_hbm, vend, VE, B * HD - v_end, 0)], v_end // 2, 4),
        ([row_piece(wo_hbm, wobuf, WO, _SLAB)], HD // _SLAB, _RUNS[4]),
        ([row_piece(wg_hbm, wgbuf, GU0, 16, early), row_piece(wu_hbm, wubuf, GU0, 16, early)],
         D // 8, _RUNS[5]),
        ([down_piece(0)], 8 * _DOWN, 1),
        ([row_piece(wg_hbm, wgbuf, GU1, 32, late), row_piece(wu_hbm, wubuf, GU1, 32, late)],
         D // 16, _RUNS[6]),
        ([down_piece(8 * _DOWN)], 8 * (_PARTS - _DOWN), 1),
    )
    u_lo = -sum(n for _, n, _ in head) // 8
    u_mid = (last - 1) * _VISITS
    u_hi = u_mid + sum(n for _, n, _ in tail) // 8

    def other_visits(at, parts, lo, hi):
        for fns, n, runs in parts:
            assert n % (runs * len(fns)) == 0

            def pair(i, fns=fns, n=n, runs=runs):
                for c in range(2):
                    k = i if len(fns) == 2 else 2 * i + c
                    turn = k >> (runs.bit_length() - 1)
                    fns[c % len(fns)]((k & (runs - 1)) * (n // len(fns) // runs) + turn, c)

            _loop(4 * jnp.clip(lo - at, 0, n // 8), 4 * jnp.clip(hi - at, 0, n // 8), pair)
            at += n // 8

    def window_visits(u):
        p = (u >> 6) + 1
        slot = jax.lax.rem(p, _NB)
        rt = (u >> 3) & 7

        def visit(i):
            cols = _ds(((u & 7) + i) * _GC, _GC)

            def piece(hbm, buf, dma_sem, pad, tile, j, skip, queue):
                at = (j & 1) * (_QTR // 2) + tile * 8
                row = p * _WIN - pad + at
                quarter, n = (j & 2) + skip, 2 - skip
                copy(
                    hbm.at[pl.ds((row >> 7) + quarter, n), _ds(row & (_QTR - 1), 8), cols],
                    buf.at[slot, pl.ds(quarter, n), _ds(at, 8), cols],
                    dma_sem.at[slot],
                    queue,
                )

            v_piece = functools.partial(piece, vt_hbm, vbuf, vsem, _V_PAD, rt)
            for j in range(4):
                piece(kt_hbm, kbuf, ksem, _K_PAD, rt, j, 0, 0)
                if j:
                    v_piece(j, 0, 1)
                else:
                    cut = jnp.logical_and(p == 1, rt < v_end // 8)
                    pl.when(cut)(lambda: v_piece(0, 1, 1))
                    pl.when(jnp.logical_not(cut))(lambda: v_piece(0, 0, 1))

        _loop(0, 4, visit)

    w_last = last * _STEPS

    def issued(w, clip=jnp.clip):
        u = 4 * clip(w, u_lo, w_last - _STEPS)
        for i, pace in enumerate(_PACE):
            u += pace * clip(w - w_last + _STEPS - i * half, 0, half)
        return clip(u + _LEAD, u_lo, u_hi)

    def issue(w):
        lo, hi = issued(w - 1), issued(w)
        pl.when(lo < 0)(lambda: other_visits(u_lo, head, lo, hi))
        pl.when(jnp.logical_and(lo >= 0, lo < u_mid))(lambda: window_visits(lo))
        pl.when(jnp.logical_and(lo >= u_mid, lo < hi))(lambda: other_visits(u_mid, tail, lo, hi))

    def owned(first_row, width):
        span = _RING * Dh
        r = jax.lax.broadcasted_iota(jnp.int32, (_RING, width), 1) + first_row
        r = jnp.where(r >= span, r - span, r)
        lo = jax.lax.broadcasted_iota(jnp.int32, (_RING, width), 0) * Dh
        return (r >= lo) & (r < lo + Dh)

    def prepare():
        copy(x_hbm, xbuf, X, 0)
        copy(wr_hbm, wrbuf, WR, 1)

        def clear(i):
            kbuf[0, i >> 3, _ds((i & 7) * 16, 16), :] = jnp.zeros((16, Sk), kbuf.dtype)

        def clear_cols(i):
            vbuf[1, 0, pl.ds(0, v_end), _ds(i * _GC, _GC)] = jnp.zeros((v_end, _GC), vbuf.dtype)
            s_scr[:, _ds(i * _GC, _GC)] = jnp.zeros((_RING, _GC), f32)
            p_scr[:, _ds(i * _GC, _GC)] = jnp.zeros((_RING, _GC), f32)

        _loop(0, _K_PAD // 16, clear)
        _loop(0, half, clear_cols)
        l_scr[...] = jnp.ones_like(l_scr)
        q_scr[:, pl.ds(0, _WIN)] = jnp.zeros((_RING, _WIN), f32)
        q_scr[:, pl.ds(B * HD, _WIN)] = jnp.zeros((_RING, _WIN), f32)

    def project(i):
        @pl.when(i == 0)
        def _():
            _wait_all(xbuf, X)
            x = xbuf[...].astype(f32)
            x_scr[...] = jnp.concatenate([x, x], axis=0)
            n_scr[...] = _layernorm(x_scr[...])
            _wait_all(wqbuf, WQ)

        def part(k):
            cols = _ds((4 * i + k) * 512, 512)
            t_scr[:, cols] = _dot(n_scr[...].astype(bf16), wqbuf[:, cols])

        _loop(0, 4, part)

    def lay_out_queries():
        span = _RING * Dh
        base, shift = _K_PAD // 128 * 128, _K_PAD % 128
        mine = owned(0, span)
        keep = jax.lax.broadcasted_iota(jnp.int32, (_RING, 128), 1) < shift

        def group(i):
            b = jax.lax.div(i, HD // span)
            q = t_scr[pl.ds(b, 1), _ds((i - b * (HD // span)) * span, span)]
            q = jnp.concatenate([jnp.where(mine, q, 0.0), jnp.zeros((_RING, 128), f32)], axis=1)
            q = pltpu.roll(q, shift, 1)
            at = pl.multiple_of(base + i * span, 128)
            q_scr[:, pl.ds(at, 128)] = jnp.where(keep, q_scr[:, pl.ds(at, 128)], q[:, :128])
            q_scr[:, pl.ds(at + 128, span)] = q[:, 128:]

        _loop(0, B * HD // span, group)

    def await_rows(buf, dma_sem, rows):
        _loop(0, rows >> 4, lambda i: _wait_all(buf.at[0, 0, pl.ds(0, 16)], dma_sem))

    def score(p, j):
        slot = jax.lax.rem(p, _NB)

        @pl.when(j == 0)
        def _():
            rows = jnp.where(p == 0, k_first, jnp.where(p == last, _K_PAD, _WIN))
            await_rows(kbuf, ksem.at[slot], rows)

        cols = _ds(j * _GC, _GC)
        q = q_scr[:, _ds(p * _WIN, _WIN)].astype(bf16)
        s_scr[:, cols] += _dot(q, kbuf[slot, :, :, cols].reshape(_WIN, _GC))

    def softmax(p):
        end = (p + 1) * _WIN - _K_PAD
        done_hi = jax.lax.div(jnp.minimum(end, B * HD), Dh)
        done_lo = jax.lax.div(jnp.maximum(end - _WIN, 0), Dh)
        ring_row = jax.lax.broadcasted_iota(jnp.int32, (_RING, 1), 0)
        done = (ring_row - done_lo) & (_RING - 1) < done_hi - done_lo
        raw = s_scr[...]
        s = raw * scale
        e = jnp.exp(s - jnp.max(s, axis=-1, keepdims=True))
        p_scr[...] = jnp.where(done, e, p_scr[...])
        l_scr[...] = jnp.where(done, jnp.sum(e, axis=-1, keepdims=True), l_scr[...])
        s_scr[...] = jnp.where(done, 0.0, raw)

    def mix(p, j):
        slot = jax.lax.rem(p, _NB)

        @pl.when(j == 0)
        def _():
            await_rows(vbuf, vsem.at[slot], jnp.where(p == 1, _WIN - v_end, _WIN))
            pv_scr[...] = jnp.zeros_like(pv_scr)

        cols = _ds(j * _GC, _GC)
        v = vbuf[slot, :, :, cols].reshape(_WIN, _GC)
        pv_scr[...] += _dot_nt(p_scr[:, cols].astype(bf16), v)

        @pl.when(j == half - 1)
        def _():
            span = _RING * Dh
            mine = owned(jax.lax.rem(p * _WIN - _V_PAD + span, span), _WIN)
            o_scr[:, _ds(p * _WIN, _WIN)] = jnp.where(mine, pv_scr[...] / l_scr[...], 0.0)

    def attend(w):
        p, j = w >> 4, w & (_STEPS - 1)
        pl.when(j < half)(lambda: score(p, j))
        pl.when(j == half)(lambda: softmax(p))
        pl.when(jnp.logical_and(j >= half, p > 0))(lambda: mix(p, j - half))

    def lay_out_values(lo, hi):
        def group(i):
            b, c = i >> 2, (i & 3) * (HD // 4)
            o = o_scr[:, pl.ds(pl.multiple_of(_WIN + i * (HD // 4), 128), HD // 4 + 128)]
            ob_scr[_ds(b * _RING, _RING), _ds(c, HD // 4)] = o[:, v_end:v_end + HD // 4]

        _loop(lo, hi, group)

    def finish_values():
        _wait_all(vend, VE)
        pv = _dot_nt(p_scr[...].astype(bf16), vend[0])
        mine = owned(_RING * Dh - v_end, v_end)
        o_scr[:, pl.ds((last + 1) * _WIN, 128)] = jnp.zeros((_RING, 128), f32)
        o_scr[:, pl.ds((last + 1) * _WIN, v_end)] = jnp.where(mine, pv / l_scr[...], 0.0)
        lay_out_values(4 * B - 2, 4 * B)
        a_scr[...] = jnp.zeros_like(a_scr)

    def merge(i):
        pl.when(i == 0)(lambda: _wait_all(wobuf, WO))
        rows = _ds(i * (HD // _PARTS), HD // _PARTS)
        a_scr[...] += _dot(ob_scr[:, rows].astype(bf16), wobuf[rows, :])

    w_end = (last + 1) * _STEPS

    def step(w):
        issue(w)
        pl.when(w == -8)(prepare)
        pl.when(jnp.logical_and(w >= -3, w < 0))(lambda: project(w + 3))
        pl.when(w == -1)(lay_out_queries)
        pl.when(jnp.logical_and(w >= 0, w < w_end))(lambda: attend(w))
        pl.when(w == w_last - 2 * _STEPS)(lambda: lay_out_values(0, 4 * B - 2))
        pl.when(w == w_end)(finish_values)
        pl.when(w >= w_end)(lambda: merge(w - w_end))

    u_caches = u_mid + (_K_PAD + _V_PAD) // 16
    for w, u in ((-3, -k_first // 16), (w_last, u_caches - _V_PAD // 16), (w_last + half, u_caches),
                 (w_end, u_caches + HD // _SLAB // 8), (w_end + _PARTS - 1, u_hi)):
        assert issued(w, lambda v, lo, hi: min(max(v, lo), hi)) >= u and _LEAD % 4 == 0
    w_lo = (u_lo - _LEAD) // 4 + 1
    _loop(0, w_end + _PARTS - w_lo, lambda i: step(i + w_lo))

    attn = jnp.sum(a_scr[...].reshape(B, _RING, D), axis=1)
    h = x_scr[...] + jnp.concatenate([attn, attn], axis=0)
    hn = _layernorm(h)
    n_scr[...] = hn
    _wait_all(wrbuf, WR)
    r = jnp.sum(hn * wrbuf[...].astype(f32).reshape(1, D), axis=-1, keepdims=True)
    route = jax.nn.sigmoid(r)

    def activate(f):
        cols = _ds(f * units, units)
        hb = n_scr[...].astype(bf16)
        gate = _dot(hb, wgbuf[:, cols])
        g_scr[:, cols] = gate * jax.nn.sigmoid(gate) * _dot(hb, wubuf[:, cols])

    def reduce(f):
        rows = _ds(f * units, units)
        _wait_all(wdbuf.at[pl.ds(0, units)], dsem.at[f])
        y_scr[...] += _dot(g_scr[:, rows].astype(bf16), wdbuf[rows, :])

    def feed_forward(i):
        for k, (cols, dma_sem) in enumerate(((early, GU0), (late, GU1))):
            @pl.when(i == k)
            def _():
                _wait_all(wgbuf.at[:, cols], dma_sem)
                _wait_all(wubuf.at[:, cols], dma_sem)

        _loop(i * _EARLY, _EARLY + i * (_PARTS - _EARLY), activate)
        _loop(i * _DOWN, _DOWN + i * (_PARTS - _DOWN), reduce)

    y_scr[...] = jnp.zeros_like(y_scr)
    _loop(0, 2, feed_forward)
    y = y_scr[...] * route
    out = h + (hn + (hn * 0.0 + y))
    out_ref[...] = out[:B].astype(out_ref.dtype)


@jax.jit
def pallas_sequential_preLN__mha_block_cached__moe_arch_mod__decode_kernel(
    A_x: jax.Array,
    A_k_cache: jax.Array,
    A_v_cache: jax.Array,
    A_wq: jax.Array,
    A_wo: jax.Array,
    B_x: jax.Array,
    B_w_r: jax.Array,
    B_w_gate: jax.Array,
    B_w_up: jax.Array,
    B_w_down: jax.Array,
):
    del B_x
    B, Sq, D = A_x.shape
    _, H, Sk, Dh = A_k_cache.shape
    F = B_w_gate.shape[1]
    HD = H * Dh
    assert (B, Sq, D, H, Sk, Dh, F) == (4, 1, 640, 32, 8 * _GC, 192, 1536)
    dt = A_k_cache.dtype
    f32 = jnp.float32

    kt = jnp.swapaxes(A_k_cache, 2, 3).reshape(B * HD // _QTR, _QTR, Sk)
    vt = jnp.swapaxes(A_v_cache, 2, 3).reshape(B * HD // _QTR, _QTR, Sk)

    out = pl.pallas_call(
        functools.partial(_body, B=B, H=H, Dh=Dh, Sk=Sk, D=D, F=F),
        in_specs=[pl.BlockSpec(memory_space=pl.ANY)] * 9,
        out_specs=pl.BlockSpec(memory_space=pltpu.VMEM),
        out_shape=jax.ShapeDtypeStruct((B, D), A_x.dtype),
        scratch_shapes=[
            pltpu.VMEM((_NB, _WIN // _QTR, _QTR, Sk), dt),
            pltpu.VMEM((_NB, _WIN // _QTR, _QTR, Sk), dt),
            pltpu.VMEM((1, _V_PAD - _WIN, Sk), dt),
            pltpu.VMEM((D, HD), dt),
            pltpu.VMEM((HD, D), dt),
            pltpu.VMEM((D, F), dt),
            pltpu.VMEM((D, F), dt),
            pltpu.VMEM((F, D), dt),
            pltpu.VMEM((B, D), dt),
            pltpu.VMEM((D,), dt),
            pltpu.VMEM((2 * B, D), f32),
            pltpu.VMEM((2 * B, D), f32),
            pltpu.VMEM((2 * B, HD), f32),
            pltpu.VMEM((_RING, B * HD + _WIN), f32),
            pltpu.VMEM((_RING, B * HD + 2 * _WIN), f32),
            pltpu.VMEM((B * _RING, HD), f32),
            pltpu.VMEM((_RING, Sk), f32),
            pltpu.VMEM((_RING, Sk), f32),
            pltpu.VMEM((_RING, 1), f32),
            pltpu.VMEM((_RING, _WIN), f32),
            pltpu.VMEM((B * _RING, D), f32),
            pltpu.VMEM((2 * B, F), f32),
            pltpu.VMEM((2 * B, D), f32),
            pltpu.SemaphoreType.DMA((_NB,)),
            pltpu.SemaphoreType.DMA((_NB,)),
            pltpu.SemaphoreType.DMA((_PARTS,)),
            pltpu.SemaphoreType.DMA((7,)),
        ],
        compiler_params=pltpu.CompilerParams(
            vmem_limit_bytes=96 * 1024 * 1024, disable_bounds_checks=_NOCHECK
        ),
    )(A_x.reshape(B, D), kt, vt, A_wq, A_wo, B_w_r, B_w_gate, B_w_up, B_w_down)
    return out.reshape(B, Sq, D)
```

```python
import functools

import jax
import jax.numpy as jnp
import jax.experimental.pallas as pl
import jax.experimental.pallas.tpu as pltpu

_EPS = 1e-5
_NOCHECK = True
_NB = 3
_WIN = 512
_QTR = 128
_GC = 1024
_VISITS = 64
_STEPS = 16
_LEAD = 16
_PACE = (3, 2, 2, 2, 4)
_SHIFT = 1
_K_PAD = 336
_V_PAD = 544
_RING = 8
_EARLY = 4
_DOWN = 0
_SLAB = 32
_PARTS = 6


def _layernorm(x):
    m = jnp.mean(x, axis=-1, keepdims=True)
    d = x - m
    v = jnp.mean(d * d, axis=-1, keepdims=True)
    return d / jnp.sqrt(v + _EPS)


def _dot(a, b):
    return jnp.dot(a, b, preferred_element_type=jnp.float32)


def _dot_nt(a, b):
    return jax.lax.dot_general(
        a, b, (((1,), (1,)), ((), ())), preferred_element_type=jnp.float32
    )


def _wait_all(buf, sem):
    pltpu.make_async_copy(buf, buf, sem).wait()


def _ds(start, size):
    return pl.ds(start if isinstance(start, int) else pl.multiple_of(start, size), size)


def _loop(lo, hi, fn):
    jax.lax.fori_loop(lo, hi, lambda i, carry: fn(i), None)


def _body(
    x_hbm, kt_hbm, vt_hbm, wq_hbm, wo_hbm, wr_hbm, wg_hbm, wu_hbm, wd_hbm,
    out_ref,
    kbuf, vbuf, vend, wqbuf, wobuf, wgbuf, wubuf, wdbuf, xbuf, wrbuf,
    x_scr, n_scr, t_scr, q_scr, o_scr, ob_scr, s_scr, p_scr, l_scr, pv_scr, a_scr, g_scr, y_scr,
    ksem, vsem, dsem, sem,
    *, B, H, Dh, Sk, D, F,
):
    HD = H * Dh
    last = B * HD // _WIN
    k_first = _WIN - _K_PAD
    v_end = _V_PAD - _WIN
    half = _STEPS // 2
    scale = Dh ** -0.5
    f32, bf16 = jnp.float32, jnp.bfloat16
    X, WR, WQ, VE, WO, GU0, GU1 = (sem.at[i] for i in range(7))

    def copy(src, dst, dma_sem, queue):
        pltpu.make_async_copy(src, dst, dma_sem).start(priority=queue)

    def window_piece(hbm, buf, dma_sem, pad, p, g, second, quarter, n, queue):
        slot = p % _NB if isinstance(p, int) else jax.lax.rem(p, _NB)
        cols = _ds((g & 7) * _GC, _GC)
        at = second * (_QTR // 2) + (g >> 3) * 8
        row = p * _WIN - pad + at
        copy(
            hbm.at[pl.ds((row >> 7) + quarter, n), _ds(row & (_QTR - 1), 8), cols],
            buf.at[slot, pl.ds(quarter, n), _ds(at, 8), cols],
            dma_sem.at[slot],
            queue,
        )

    def cache_piece(hbm, buf, dma_sem, row, buf_row):
        def piece(g, queue):
            r, cols = (g >> 2) * 8, _ds((g & 3) * 2 * _GC, 2 * _GC)
            src, dst = row + r, buf_row + r
            copy(
                hbm.at[src >> 7, _ds(src & (_QTR - 1), 8), cols],
                buf.at[dst >> 7, _ds(dst & (_QTR - 1), 8), cols],
                dma_sem,
                queue,
            )

        return piece

    def wq_piece(g, queue):
        row = g * 171 >> 9
        where = (_ds(row * 8, 8), _ds((g - 3 * row) * 2 * _GC, 2 * _GC))
        copy(wq_hbm.at[where], wqbuf.at[where], WQ, queue)

    def row_piece(hbm, buf, dma_sem, rows, cols=slice(None)):
        def piece(g, queue):
            where = (_ds(g * rows, rows), cols)
            copy(hbm.at[where], buf.at[where], dma_sem, queue)

        return piece

    def down_piece(first):
        def piece(g, queue):
            rows = _ds((first + g) * _SLAB, _SLAB)
            copy(wd_hbm.at[rows], wdbuf.at[rows], dsem.at[(first + g) >> 3], queue)

        return piece

    end_slot = last % _NB
    units = F // _PARTS
    early, late = pl.ds(0, _EARLY * units), pl.ds(_EARLY * units, F - _EARLY * units)
    head = (
        ([wq_piece], D // 8 * HD // (2 * _GC), 16),
        ([cache_piece(kt_hbm, kbuf.at[0], ksem.at[0], 0, _K_PAD)], k_first // 2, 8),
    )
    tail = (
        ([cache_piece(kt_hbm, kbuf.at[end_slot], ksem.at[end_slot], B * HD - _K_PAD, 0)],
         _K_PAD // 2, 8),
        ([cache_piece(vt_hbm, vbuf.at[end_slot], vsem.at[end_slot], B * HD - _V_PAD, 0)],
         _WIN // 2, 16),
        ([cache_piece(vt_hbm, vend, VE, B * HD - v_end, 0)], v_end // 2, 4),
        ([row_piece(wo_hbm, wobuf, WO, _SLAB)], HD // _SLAB, 8),
        ([row_piece(wg_hbm, wgbuf, GU0, 16, early), row_piece(wu_hbm, wubuf, GU0, 16, early)],
         D // 8, 4),
        ([down_piece(0)], 8 * _DOWN, 1),
        ([row_piece(wg_hbm, wgbuf, GU1, 32, late), row_piece(wu_hbm, wubuf, GU1, 32, late)],
         D // 16, 4),
        ([down_piece(8 * _DOWN)], 8 * (_PARTS - _DOWN), 1),
    )
    u_lo = -sum(n for _, n, _ in head) // 8
    u_mid = (last - 1) * _VISITS
    u_hi = u_mid + sum(n for _, n, _ in tail) // 8

    def other_visits(at, parts, lo, hi):
        for fns, n, runs in parts:
            assert n % (runs * len(fns)) == 0

            def pair(i, fns=fns, n=n, runs=runs):
                for c in range(2):
                    k = i if len(fns) == 2 else 2 * i + c
                    turn = k >> (runs.bit_length() - 1)
                    fns[c % len(fns)]((k & (runs - 1)) * (n // len(fns) // runs) + turn, c)

            _loop(4 * jnp.clip(lo - at, 0, n // 8), 4 * jnp.clip(hi - at, 0, n // 8), pair)
            at += n // 8

    def window_visits(u):
        p = (u >> 6) + 1
        k_piece = functools.partial(window_piece, kt_hbm, kbuf, ksem, _K_PAD, p)
        v_piece = functools.partial(window_piece, vt_hbm, vbuf, vsem, _V_PAD, p)

        def visit(i):
            quarter = (i & 1) * 2
            for d in range(2):
                g = (u + (i & 2) + d + _SHIFT) & (_VISITS - 1)
                cut = (p == 1) & (quarter == 0) & (g < v_end)
                k_piece(g, 0, quarter, 2, 0)
                pl.when(cut)(lambda: v_piece(g, 0, 1, 1, 1))
                pl.when(jnp.logical_not(cut))(lambda: v_piece(g, 0, quarter, 2, 1))
                k_piece(g, 1, quarter, 2, 0)
                v_piece(g, 1, quarter, 2, 1)

        _loop(0, 4, visit)

    w_last = last * _STEPS

    def issued(w, clip=jnp.clip):
        u = 4 * clip(w, u_lo, w_last - _STEPS)
        for i, pace in enumerate(_PACE):
            u += pace * clip(w - w_last + _STEPS - i * half, 0, half)
        return clip(u + _LEAD, u_lo, u_hi)

    def issue(w):
        lo, hi = issued(w - 1), issued(w)
        pl.when(lo < 0)(lambda: other_visits(u_lo, head, lo, hi))
        pl.when(jnp.logical_and(lo >= 0, lo < u_mid))(lambda: window_visits(lo))
        pl.when(jnp.logical_and(lo >= u_mid, lo < hi))(lambda: other_visits(u_mid, tail, lo, hi))

    def owned(first_row, width):
        span = _RING * Dh
        r = jax.lax.broadcasted_iota(jnp.int32, (_RING, width), 1) + first_row
        r = jnp.where(r >= span, r - span, r)
        lo = jax.lax.broadcasted_iota(jnp.int32, (_RING, width), 0) * Dh
        return (r >= lo) & (r < lo + Dh)

    def prepare():
        copy(x_hbm, xbuf, X, 0)
        copy(wr_hbm, wrbuf, WR, 1)

        def clear(i):
            kbuf[0, i >> 3, _ds((i & 7) * 16, 16), :] = jnp.zeros((16, Sk), kbuf.dtype)

        def clear_cols(i):
            vbuf[1, 0, pl.ds(0, v_end), _ds(i * _GC, _GC)] = jnp.zeros((v_end, _GC), vbuf.dtype)
            s_scr[:, _ds(i * _GC, _GC)] = jnp.zeros((_RING, _GC), f32)
            p_scr[:, _ds(i * _GC, _GC)] = jnp.zeros((_RING, _GC), f32)

        _loop(0, _K_PAD // 16, clear)
        _loop(0, half, clear_cols)
        l_scr[...] = jnp.ones_like(l_scr)
        q_scr[:, pl.ds(0, _WIN)] = jnp.zeros((_RING, _WIN), f32)
        q_scr[:, pl.ds(B * HD, _WIN)] = jnp.zeros((_RING, _WIN), f32)

    def project(i):
        @pl.when(i == 0)
        def _():
            _wait_all(xbuf, X)
            x = xbuf[...].astype(f32)
            x_scr[...] = jnp.concatenate([x, x], axis=0)
            n_scr[...] = _layernorm(x_scr[...])
            _wait_all(wqbuf, WQ)

        def part(k):
            cols = _ds((4 * i + k) * 512, 512)
            t_scr[:, cols] = _dot(n_scr[...].astype(bf16), wqbuf[:, cols])

        _loop(0, 4, part)

    def lay_out_queries():
        span = _RING * Dh
        base, shift = _K_PAD // 128 * 128, _K_PAD % 128
        mine = owned(0, span)
        keep = jax.lax.broadcasted_iota(jnp.int32, (_RING, 128), 1) < shift

        def group(i):
            b = jax.lax.div(i, HD // span)
            q = t_scr[pl.ds(b, 1), _ds((i - b * (HD // span)) * span, span)]
            q = jnp.concatenate([jnp.where(mine, q, 0.0), jnp.zeros((_RING, 128), f32)], axis=1)
            q = pltpu.roll(q, shift, 1)
            at = pl.multiple_of(base + i * span, 128)
            q_scr[:, pl.ds(at, 128)] = jnp.where(keep, q_scr[:, pl.ds(at, 128)], q[:, :128])
            q_scr[:, pl.ds(at + 128, span)] = q[:, 128:]

        _loop(0, B * HD // span, group)

    def await_rows(buf, dma_sem, rows):
        _loop(0, rows >> 4, lambda i: _wait_all(buf.at[0, 0, pl.ds(0, 16)], dma_sem))

    def score(p, j):
        slot = jax.lax.rem(p, _NB)

        @pl.when(j == 0)
        def _():
            rows = jnp.where(p == 0, k_first, jnp.where(p == last, _K_PAD, _WIN))
            await_rows(kbuf, ksem.at[slot], rows)

        cols = _ds(j * _GC, _GC)
        q = q_scr[:, _ds(p * _WIN, _WIN)].astype(bf16)
        s_scr[:, cols] += _dot(q, kbuf[slot, :, :, cols].reshape(_WIN, _GC))

    def softmax(p):
        end = (p + 1) * _WIN - _K_PAD
        done_hi = jax.lax.div(jnp.minimum(end, B * HD), Dh)
        done_lo = jax.lax.div(jnp.maximum(end - _WIN, 0), Dh)
        ring_row = jax.lax.broadcasted_iota(jnp.int32, (_RING, 1), 0)
        done = (ring_row - done_lo) & (_RING - 1) < done_hi - done_lo
        raw = s_scr[...]
        s = raw * scale
        e = jnp.exp(s - jnp.max(s, axis=-1, keepdims=True))
        p_scr[...] = jnp.where(done, e, p_scr[...])
        l_scr[...] = jnp.where(done, jnp.sum(e, axis=-1, keepdims=True), l_scr[...])
        s_scr[...] = jnp.where(done, 0.0, raw)

    def mix(p, j):
        slot = jax.lax.rem(p, _NB)

        @pl.when(j == 0)
        def _():
            await_rows(vbuf, vsem.at[slot], jnp.where(p == 1, _WIN - v_end, _WIN))
            pv_scr[...] = jnp.zeros_like(pv_scr)

        cols = _ds(j * _GC, _GC)
        v = vbuf[slot, :, :, cols].reshape(_WIN, _GC)
        pv_scr[...] += _dot_nt(p_scr[:, cols].astype(bf16), v)

        @pl.when(j == half - 1)
        def _():
            span = _RING * Dh
            mine = owned(jax.lax.rem(p * _WIN - _V_PAD + span, span), _WIN)
            o_scr[:, _ds(p * _WIN, _WIN)] = jnp.where(mine, pv_scr[...] / l_scr[...], 0.0)

    def attend(w):
        p, j = w >> 4, w & (_STEPS - 1)
        pl.when(j < half)(lambda: score(p, j))
        pl.when(j == half)(lambda: softmax(p))
        pl.when(jnp.logical_and(j >= half, p > 0))(lambda: mix(p, j - half))

    def lay_out_values(lo, hi):
        def group(i):
            b, c = i >> 2, (i & 3) * (HD // 4)
            o = o_scr[:, pl.ds(pl.multiple_of(_WIN + i * (HD // 4), 128), HD // 4 + 128)]
            ob_scr[_ds(b * _RING, _RING), _ds(c, HD // 4)] = o[:, v_end:v_end + HD // 4]

        _loop(lo, hi, group)

    def finish_values():
        _wait_all(vend, VE)
        pv = _dot_nt(p_scr[...].astype(bf16), vend[0])
        mine = owned(_RING * Dh - v_end, v_end)
        o_scr[:, pl.ds((last + 1) * _WIN, 128)] = jnp.zeros((_RING, 128), f32)
        o_scr[:, pl.ds((last + 1) * _WIN, v_end)] = jnp.where(mine, pv / l_scr[...], 0.0)
        lay_out_values(4 * B - 2, 4 * B)
        a_scr[...] = jnp.zeros_like(a_scr)

    def merge(i):
        pl.when(i == 0)(lambda: _wait_all(wobuf, WO))
        rows = _ds(i * (HD // _PARTS), HD // _PARTS)
        a_scr[...] += _dot(ob_scr[:, rows].astype(bf16), wobuf[rows, :])

    w_end = (last + 1) * _STEPS

    def step(w):
        issue(w)
        pl.when(w == -8)(prepare)
        pl.when(jnp.logical_and(w >= -3, w < 0))(lambda: project(w + 3))
        pl.when(w == -1)(lay_out_queries)
        pl.when(jnp.logical_and(w >= 0, w < w_end))(lambda: attend(w))
        pl.when(w == w_last - 2 * _STEPS)(lambda: lay_out_values(0, 4 * B - 2))
        pl.when(w == w_end)(finish_values)
        pl.when(w >= w_end)(lambda: merge(w - w_end))

    u_caches = u_mid + (_K_PAD + _V_PAD) // 16
    for w, u in ((-3, -k_first // 16), (w_last, u_caches - _V_PAD // 16), (w_last + half, u_caches),
                 (w_end, u_caches + HD // _SLAB // 8), (w_end + _PARTS - 1, u_hi)):
        assert issued(w, lambda v, lo, hi: min(max(v, lo), hi)) >= u and _LEAD % 4 == 0
    w_lo = (u_lo - _LEAD) // 4 + 1
    _loop(0, w_end + _PARTS - w_lo, lambda i: step(i + w_lo))

    attn = jnp.sum(a_scr[...].reshape(B, _RING, D), axis=1)
    h = x_scr[...] + jnp.concatenate([attn, attn], axis=0)
    hn = _layernorm(h)
    n_scr[...] = hn
    _wait_all(wrbuf, WR)
    r = jnp.sum(hn * wrbuf[...].astype(f32).reshape(1, D), axis=-1, keepdims=True)
    route = jax.nn.sigmoid(r)

    def activate(f):
        cols = _ds(f * units, units)
        hb = n_scr[...].astype(bf16)
        gate = _dot(hb, wgbuf[:, cols])
        g_scr[:, cols] = gate * jax.nn.sigmoid(gate) * _dot(hb, wubuf[:, cols])

    def reduce(f):
        rows = _ds(f * units, units)
        _wait_all(wdbuf.at[pl.ds(0, units)], dsem.at[f])
        y_scr[...] += _dot(g_scr[:, rows].astype(bf16), wdbuf[rows, :])

    def feed_forward(i):
        for k, (cols, dma_sem) in enumerate(((early, GU0), (late, GU1))):
            @pl.when(i == k)
            def _():
                _wait_all(wgbuf.at[:, cols], dma_sem)
                _wait_all(wubuf.at[:, cols], dma_sem)

        _loop(i * _EARLY, _EARLY + i * (_PARTS - _EARLY), activate)
        _loop(i * _DOWN, _DOWN + i * (_PARTS - _DOWN), reduce)

    y_scr[...] = jnp.zeros_like(y_scr)
    _loop(0, 2, feed_forward)
    y = y_scr[...] * route
    out = h + (hn + (hn * 0.0 + y))
    out_ref[...] = out[:B].astype(out_ref.dtype)


@jax.jit
def pallas_sequential_preLN__mha_block_cached__moe_arch_mod__decode_kernel(
    A_x: jax.Array,
    A_k_cache: jax.Array,
    A_v_cache: jax.Array,
    A_wq: jax.Array,
    A_wo: jax.Array,
    B_x: jax.Array,
    B_w_r: jax.Array,
    B_w_gate: jax.Array,
    B_w_up: jax.Array,
    B_w_down: jax.Array,
):
    del B_x
    B, Sq, D = A_x.shape
    _, H, Sk, Dh = A_k_cache.shape
    F = B_w_gate.shape[1]
    HD = H * Dh
    assert (B, Sq, D, H, Sk, Dh, F) == (4, 1, 640, 32, 8 * _GC, 192, 1536)
    dt = A_k_cache.dtype
    f32 = jnp.float32

    kt = jnp.swapaxes(A_k_cache, 2, 3).reshape(B * HD // _QTR, _QTR, Sk)
    vt = jnp.swapaxes(A_v_cache, 2, 3).reshape(B * HD // _QTR, _QTR, Sk)

    out = pl.pallas_call(
        functools.partial(_body, B=B, H=H, Dh=Dh, Sk=Sk, D=D, F=F),
        in_specs=[pl.BlockSpec(memory_space=pl.ANY)] * 9,
        out_specs=pl.BlockSpec(memory_space=pltpu.VMEM),
        out_shape=jax.ShapeDtypeStruct((B, D), A_x.dtype),
        scratch_shapes=[
            pltpu.VMEM((_NB, _WIN // _QTR, _QTR, Sk), dt),
            pltpu.VMEM((_NB, _WIN // _QTR, _QTR, Sk), dt),
            pltpu.VMEM((1, _V_PAD - _WIN, Sk), dt),
            pltpu.VMEM((D, HD), dt),
            pltpu.VMEM((HD, D), dt),
            pltpu.VMEM((D, F), dt),
            pltpu.VMEM((D, F), dt),
            pltpu.VMEM((F, D), dt),
            pltpu.VMEM((B, D), dt),
            pltpu.VMEM((D,), dt),
            pltpu.VMEM((2 * B, D), f32),
            pltpu.VMEM((2 * B, D), f32),
            pltpu.VMEM((2 * B, HD), f32),
            pltpu.VMEM((_RING, B * HD + _WIN), f32),
            pltpu.VMEM((_RING, B * HD + 2 * _WIN), f32),
            pltpu.VMEM((B * _RING, HD), f32),
            pltpu.VMEM((_RING, Sk), f32),
            pltpu.VMEM((_RING, Sk), f32),
            pltpu.VMEM((_RING, 1), f32),
            pltpu.VMEM((_RING, _WIN), f32),
            pltpu.VMEM((B * _RING, D), f32),
            pltpu.VMEM((2 * B, F), f32),
            pltpu.VMEM((2 * B, D), f32),
            pltpu.SemaphoreType.DMA((_NB,)),
            pltpu.SemaphoreType.DMA((_NB,)),
            pltpu.SemaphoreType.DMA((_PARTS,)),
            pltpu.SemaphoreType.DMA((7,)),
        ],
        compiler_params=pltpu.CompilerParams(
            vmem_limit_bytes=96 * 1024 * 1024, disable_bounds_checks=_NOCHECK
        ),
    )(A_x.reshape(B, D), kt, vt, A_wq, A_wo, B_w_r, B_w_gate, B_w_up, B_w_down)
    return out.reshape(B, Sq, D)
```

```python
import functools

import jax
import jax.numpy as jnp
import jax.experimental.pallas as pl
import jax.experimental.pallas.tpu as pltpu

_EPS = 1e-5
_NB = 3
_WIN = 512
_QTR = 128
_GC = 1024
_VISITS = 64
_STEPS = 16
_LEAD = 16
_PACE = (3, 2, 2, 2, 4)
_K_START = 1
_V_START = 37
_K_PAD = 336
_V_PAD = 544
_RING = 8
_SLAB = 32
_PARTS = 6
_EARLY = 4


def _layernorm(x):
    m = jnp.mean(x, axis=-1, keepdims=True)
    d = x - m
    v = jnp.mean(d * d, axis=-1, keepdims=True)
    return d / jnp.sqrt(v + _EPS)


def _dot(a, b):
    return jnp.dot(a, b, preferred_element_type=jnp.float32)


def _dot_nt(a, b):
    return jax.lax.dot_general(
        a, b, (((1,), (1,)), ((), ())), preferred_element_type=jnp.float32
    )


def _wait_all(buf, sem):
    pltpu.make_async_copy(buf, buf, sem).wait()


def _ds(start, size):
    return pl.ds(start if isinstance(start, int) else pl.multiple_of(start, size), size)


def _loop(lo, hi, fn):
    jax.lax.fori_loop(lo, hi, lambda i, carry: fn(i), None)


def _body(
    x_hbm, kt_hbm, vt_hbm, wq_hbm, wo_hbm, wr_hbm, wg_hbm, wu_hbm, wd_hbm,
    out_ref,
    kbuf, vbuf, vend, wqbuf, wobuf, wgbuf, wubuf, wdbuf, xbuf, wrbuf,
    x_scr, n_scr, t_scr, q_scr, o_scr, ob_scr, s_scr, p_scr, l_scr, pv_scr, a_scr, g_scr, y_scr,
    ksem, vsem, dsem, sem,
    *, B, H, Dh, Sk, D, F,
):
    HD = H * Dh
    last = B * HD // _WIN
    k_first = _WIN - _K_PAD
    v_end = _V_PAD - _WIN
    half = _STEPS // 2
    scale = Dh ** -0.5
    f32, bf16 = jnp.float32, jnp.bfloat16
    X, WR, WQ, VE, WO, GU0, GU1 = (sem.at[i] for i in range(7))

    def copy(src, dst, dma_sem, queue):
        pltpu.make_async_copy(src, dst, dma_sem).start(priority=queue)

    def window_piece(hbm, buf, dma_sem, pad, p, g, second, quarter, n, queue):
        slot = jax.lax.rem(p, _NB)
        cols = _ds((g & 7) * _GC, _GC)
        at = second * (_QTR // 2) + (g >> 3) * 8
        row = p * _WIN - pad + at
        copy(
            hbm.at[pl.ds((row >> 7) + quarter, n), _ds(row & (_QTR - 1), 8), cols],
            buf.at[slot, pl.ds(quarter, n), _ds(at, 8), cols],
            dma_sem.at[slot],
            queue,
        )

    def cache_piece(hbm, buf, dma_sem, row, buf_row):
        def piece(g, queue):
            r, cols = (g >> 2) * 8, _ds((g & 3) * 2 * _GC, 2 * _GC)
            src, dst = row + r, buf_row + r
            copy(
                hbm.at[src >> 7, _ds(src & (_QTR - 1), 8), cols],
                buf.at[dst >> 7, _ds(dst & (_QTR - 1), 8), cols],
                dma_sem,
                queue,
            )

        return piece

    def wq_piece(g, queue):
        row = g * 171 >> 9
        where = (_ds(row * 8, 8), _ds((g - 3 * row) * 2 * _GC, 2 * _GC))
        copy(wq_hbm.at[where], wqbuf.at[where], WQ, queue)

    def row_piece(hbm, buf, dma_sem, rows, cols=slice(None)):
        def piece(g, queue):
            where = (_ds(g * rows, rows), cols)
            copy(hbm.at[where], buf.at[where], dma_sem, queue)

        return piece

    def down_piece(g, queue):
        rows = _ds(g * _SLAB, _SLAB)
        copy(wd_hbm.at[rows], wdbuf.at[rows], dsem.at[g >> 3], queue)

    end_slot = last % _NB
    units = F // _PARTS
    early, late = pl.ds(0, _EARLY * units), pl.ds(_EARLY * units, F - _EARLY * units)
    head = (
        ([wq_piece], D // 8 * HD // (2 * _GC), 16),
        ([cache_piece(kt_hbm, kbuf.at[0], ksem.at[0], 0, _K_PAD)], k_first // 2, 8),
    )
    tail = (
        ([cache_piece(kt_hbm, kbuf.at[end_slot], ksem.at[end_slot], B * HD - _K_PAD, 0)],
         _K_PAD // 2, 8),
        ([cache_piece(vt_hbm, vbuf.at[end_slot], vsem.at[end_slot], B * HD - _V_PAD, 0)],
         _WIN // 2, 16),
        ([cache_piece(vt_hbm, vend, VE, B * HD - v_end, 0)], v_end // 2, 4),
        ([row_piece(wo_hbm, wobuf, WO, _SLAB)], HD // _SLAB, 8),
        ([row_piece(wg_hbm, wgbuf, GU0, 16, early), row_piece(wu_hbm, wubuf, GU0, 16, early)],
         D // 8, 4),
        ([row_piece(wg_hbm, wgbuf, GU1, 32, late), row_piece(wu_hbm, wubuf, GU1, 32, late)],
         D // 16, 4),
        ([down_piece], F // _SLAB, 1),
    )
    u_lo = -sum(n for _, n, _ in head) // 8
    u_mid = (last - 1) * _VISITS
    u_hi = u_mid + sum(n for _, n, _ in tail) // 8

    def other_visits(at, parts, lo, hi):
        for fns, n, runs in parts:
            assert n % (runs * len(fns)) == 0

            def pair(i, fns=fns, n=n, runs=runs):
                for c in range(2):
                    k = i if len(fns) == 2 else 2 * i + c
                    turn = k >> (runs.bit_length() - 1)
                    fns[c % len(fns)]((k & (runs - 1)) * (n // len(fns) // runs) + turn, c)

            _loop(4 * jnp.clip(lo - at, 0, n // 8), 4 * jnp.clip(hi - at, 0, n // 8), pair)
            at += n // 8

    def window_visits(u):
        p = (u >> 6) + 1
        k_piece = functools.partial(window_piece, kt_hbm, kbuf, ksem, _K_PAD, p)
        v_piece = functools.partial(window_piece, vt_hbm, vbuf, vsem, _V_PAD, p)

        def visit(i):
            quarter = (i & 1) * 2
            for d in range(2):
                gk = (u + (i & 2) + d + _K_START) & (_VISITS - 1)
                gv = (u + (i & 2) + d + _V_START) & (_VISITS - 1)
                cut = (p == 1) & (quarter == 0) & (gv < v_end)
                k_piece(gk, 0, quarter, 2, 0)
                pl.when(cut)(lambda: v_piece(gv, 0, 1, 1, 1))
                pl.when(jnp.logical_not(cut))(lambda: v_piece(gv, 0, quarter, 2, 1))
                k_piece(gk, 1, quarter, 2, 0)
                v_piece(gv, 1, quarter, 2, 1)

        _loop(0, 4, visit)

    w_last = last * _STEPS

    def issued(w, clip=jnp.clip):
        u = 4 * clip(w, u_lo, w_last - _STEPS)
        for i, pace in enumerate(_PACE):
            u += pace * clip(w - w_last + _STEPS - i * half, 0, half)
        return clip(u + _LEAD, u_lo + 1, u_hi)

    def issue(w):
        lo, hi = issued(w - 1), issued(w)
        pl.when(lo < 0)(lambda: other_visits(u_lo, head, lo, hi))
        pl.when(jnp.logical_and(lo >= 0, lo < u_mid))(lambda: window_visits(lo))
        pl.when(jnp.logical_and(lo >= u_mid, lo < hi))(lambda: other_visits(u_mid, tail, lo, hi))

    def owned(first_row, width):
        span = _RING * Dh
        r = jax.lax.broadcasted_iota(jnp.int32, (_RING, width), 1) + first_row
        r = jnp.where(r >= span, r - span, r)
        lo = jax.lax.broadcasted_iota(jnp.int32, (_RING, width), 0) * Dh
        return (r >= lo) & (r < lo + Dh)

    def prepare():
        copy(x_hbm, xbuf, X, 0)
        copy(wr_hbm, wrbuf, WR, 1)

        def clear(i):
            kbuf[0, i >> 3, _ds((i & 7) * 16, 16), :] = jnp.zeros((16, Sk), kbuf.dtype)

        def clear_cols(i):
            vbuf[1, 0, pl.ds(0, v_end), _ds(i * _GC, _GC)] = jnp.zeros((v_end, _GC), vbuf.dtype)
            s_scr[:, _ds(i * _GC, _GC)] = jnp.zeros((_RING, _GC), f32)
            p_scr[:, _ds(i * _GC, _GC)] = jnp.zeros((_RING, _GC), f32)

        _loop(0, _K_PAD // 16, clear)
        _loop(0, half, clear_cols)
        l_scr[...] = jnp.ones_like(l_scr)
        q_scr[:, pl.ds(0, _WIN)] = jnp.zeros((_RING, _WIN), f32)
        q_scr[:, pl.ds(B * HD, _WIN)] = jnp.zeros((_RING, _WIN), f32)

    def project(i):
        @pl.when(i == 0)
        def _():
            _wait_all(xbuf, X)
            x = xbuf[...].astype(f32)
            x_scr[...] = jnp.concatenate([x, x], axis=0)
            n_scr[...] = _layernorm(x_scr[...])
            _wait_all(wqbuf, WQ)

        def part(k):
            cols = _ds((4 * i + k) * 512, 512)
            t_scr[:, cols] = _dot(n_scr[...].astype(bf16), wqbuf[:, cols])

        _loop(0, 4, part)

    def lay_out_queries():
        span = _RING * Dh
        base, shift = _K_PAD // 128 * 128, _K_PAD % 128
        mine = owned(0, span)
        keep = jax.lax.broadcasted_iota(jnp.int32, (_RING, 128), 1) < shift

        def group(i):
            b = jax.lax.div(i, HD // span)
            q = t_scr[pl.ds(b, 1), _ds((i - b * (HD // span)) * span, span)]
            q = jnp.concatenate([jnp.where(mine, q, 0.0), jnp.zeros((_RING, 128), f32)], axis=1)
            q = pltpu.roll(q, shift, 1)
            at = pl.multiple_of(base + i * span, 128)
            q_scr[:, pl.ds(at, 128)] = jnp.where(keep, q_scr[:, pl.ds(at, 128)], q[:, :128])
            q_scr[:, pl.ds(at + 128, span)] = q[:, 128:]

        _loop(0, B * HD // span, group)

    def await_rows(buf, dma_sem, slot, lo, hi):
        def rows(i):
            _wait_all(buf.at[slot, i >> 3, _ds((i & 7) * 16, 16)], dma_sem.at[slot])

        _loop(lo >> 4, hi >> 4, rows)

    def score(p, j):
        slot = jax.lax.rem(p, _NB)

        @pl.when(j == 0)
        def _():
            lo, hi = jnp.where(p == 0, _K_PAD, 0), jnp.where(p == last, _K_PAD, _WIN)
            await_rows(kbuf, ksem, slot, lo, hi)

        cols = _ds(j * _GC, _GC)
        q = q_scr[:, _ds(p * _WIN, _WIN)].astype(bf16)
        s_scr[:, cols] += _dot(q, kbuf[slot, :, :, cols].reshape(_WIN, _GC))

    def softmax(p):
        end = (p + 1) * _WIN - _K_PAD
        done_hi = jax.lax.div(jnp.minimum(end, B * HD), Dh)
        done_lo = jax.lax.div(jnp.maximum(end - _WIN, 0), Dh)
        ring_row = jax.lax.broadcasted_iota(jnp.int32, (_RING, 1), 0)
        done = (ring_row - done_lo) & (_RING - 1) < done_hi - done_lo
        raw = s_scr[...]
        s = raw * scale
        e = jnp.exp(s - jnp.max(s, axis=-1, keepdims=True))
        p_scr[...] = jnp.where(done, e, p_scr[...])
        l_scr[...] = jnp.where(done, jnp.sum(e, axis=-1, keepdims=True), l_scr[...])
        s_scr[...] = jnp.where(done, 0.0, raw)

    def mix(p, j):
        slot = jax.lax.rem(p, _NB)

        @pl.when(j == 0)
        def _():
            await_rows(vbuf, vsem, slot, jnp.where(p == 1, v_end, 0), _WIN)
            pv_scr[...] = jnp.zeros_like(pv_scr)

        cols = _ds(j * _GC, _GC)
        v = vbuf[slot, :, :, cols].reshape(_WIN, _GC)
        pv_scr[...] += _dot_nt(p_scr[:, cols].astype(bf16), v)

        @pl.when(j == half - 1)
        def _():
            span = _RING * Dh
            mine = owned(jax.lax.rem(p * _WIN - _V_PAD + span, span), _WIN)
            o_scr[:, _ds(p * _WIN, _WIN)] = jnp.where(mine, pv_scr[...] / l_scr[...], 0.0)

    def attend(w):
        p, j = w >> 4, w & (_STEPS - 1)
        pl.when(j < half)(lambda: score(p, j))
        pl.when(j == half)(lambda: softmax(p))
        pl.when(jnp.logical_and(j >= half, p > 0))(lambda: mix(p, j - half))

    def lay_out_values(lo, hi):
        def group(i):
            b, c = i >> 2, (i & 3) * (HD // 4)
            o = o_scr[:, pl.ds(pl.multiple_of(_WIN + i * (HD // 4), 128), HD // 4 + 128)]
            ob_scr[_ds(b * _RING, _RING), _ds(c, HD // 4)] = o[:, v_end:v_end + HD // 4]

        _loop(lo, hi, group)

    def finish_values():
        _wait_all(vend, VE)
        pv = _dot_nt(p_scr[...].astype(bf16), vend[0])
        mine = owned(_RING * Dh - v_end, v_end)
        o_scr[:, pl.ds((last + 1) * _WIN, 128)] = jnp.zeros((_RING, 128), f32)
        o_scr[:, pl.ds((last + 1) * _WIN, v_end)] = jnp.where(mine, pv / l_scr[...], 0.0)
        lay_out_values(4 * B - 2, 4 * B)
        a_scr[...] = jnp.zeros_like(a_scr)

    def merge(i):
        pl.when(i == 0)(lambda: _wait_all(wobuf, WO))
        rows = _ds(i * (HD // _PARTS), HD // _PARTS)
        a_scr[...] += _dot(ob_scr[:, rows].astype(bf16), wobuf[rows, :])

    w_end = (last + 1) * _STEPS

    def step(w):
        issue(w)
        pl.when(w == -8)(prepare)
        pl.when(jnp.logical_and(w >= -3, w < 0))(lambda: project(w + 3))
        pl.when(w == -1)(lay_out_queries)
        pl.when(jnp.logical_and(w >= 0, w < w_end))(lambda: attend(w))
        pl.when(w == w_last - 2 * _STEPS)(lambda: lay_out_values(0, 4 * B - 2))
        pl.when(w == w_end)(finish_values)
        pl.when(w >= w_end)(lambda: merge(w - w_end))

    u_caches = u_mid + (_K_PAD + _V_PAD) // 16
    for w, u in ((-3, -k_first // 16), (w_last, u_caches - _V_PAD // 16), (w_last + half, u_caches),
                 (w_end, u_caches + HD // _SLAB // 8), (w_end + _PARTS - 1, u_hi)):
        assert issued(w, lambda v, lo, hi: min(max(v, lo), hi)) >= u and _LEAD % 4 == 0
    for k in range(8):
        wq_piece(k * (head[0][1] // head[0][2]), k % 2)
    w_lo = (u_lo + 1 - _LEAD) // 4 + 1
    _loop(0, w_end + _PARTS - w_lo, lambda i: step(i + w_lo))

    attn = jnp.sum(a_scr[...].reshape(B, _RING, D), axis=1)
    h = x_scr[...] + jnp.concatenate([attn, attn], axis=0)
    hn = _layernorm(h)
    n_scr[...] = hn
    _wait_all(wrbuf, WR)
    r = jnp.sum(hn * wrbuf[...].astype(f32).reshape(1, D), axis=-1, keepdims=True)
    route = jax.nn.sigmoid(r)

    def activate(f):
        cols = _ds(f * units, units)
        hb = n_scr[...].astype(bf16)
        gate = _dot(hb, wgbuf[:, cols])
        g_scr[:, cols] = gate * jax.nn.sigmoid(gate) * _dot(hb, wubuf[:, cols])

    def reduce(f):
        rows = _ds(f * units, units)
        _wait_all(wdbuf.at[rows], dsem.at[f])
        y_scr[...] += _dot(g_scr[:, rows].astype(bf16), wdbuf[rows, :])

    def feed_forward(i):
        for k, (cols, dma_sem) in enumerate(((early, GU0), (late, GU1))):
            @pl.when(i == k)
            def _():
                _wait_all(wgbuf.at[:, cols], dma_sem)
                _wait_all(wubuf.at[:, cols], dma_sem)

        _loop(i * _EARLY, _EARLY + i * (_PARTS - _EARLY), activate)

    _loop(0, 2, feed_forward)
    y_scr[...] = jnp.zeros_like(y_scr)
    _loop(0, _PARTS, reduce)
    y = y_scr[...] * route
    out = h + (hn + (hn * 0.0 + y))
    out_ref[...] = out[:B].astype(out_ref.dtype)


@jax.jit
def pallas_sequential_preLN__mha_block_cached__moe_arch_mod__decode_kernel(
    A_x: jax.Array,
    A_k_cache: jax.Array,
    A_v_cache: jax.Array,
    A_wq: jax.Array,
    A_wo: jax.Array,
    B_x: jax.Array,
    B_w_r: jax.Array,
    B_w_gate: jax.Array,
    B_w_up: jax.Array,
    B_w_down: jax.Array,
):
    del B_x
    B, Sq, D = A_x.shape
    _, H, Sk, Dh = A_k_cache.shape
    F = B_w_gate.shape[1]
    HD = H * Dh
    assert (B, Sq, D, H, Sk, Dh, F) == (4, 1, 640, 32, 8 * _GC, 192, 1536)
    dt = A_k_cache.dtype
    f32 = jnp.float32

    kt = jnp.swapaxes(A_k_cache, 2, 3).reshape(B * HD // _QTR, _QTR, Sk)
    vt = jnp.swapaxes(A_v_cache, 2, 3).reshape(B * HD // _QTR, _QTR, Sk)

    out = pl.pallas_call(
        functools.partial(_body, B=B, H=H, Dh=Dh, Sk=Sk, D=D, F=F),
        in_specs=[pl.BlockSpec(memory_space=pl.ANY)] * 9,
        out_specs=pl.BlockSpec(memory_space=pltpu.VMEM),
        out_shape=jax.ShapeDtypeStruct((B, D), A_x.dtype),
        scratch_shapes=[
            pltpu.VMEM((_NB, _WIN // _QTR, _QTR, Sk), dt),
            pltpu.VMEM((_NB, _WIN // _QTR, _QTR, Sk), dt),
            pltpu.VMEM((1, _V_PAD - _WIN, Sk), dt),
            pltpu.VMEM((D, HD), dt),
            pltpu.VMEM((HD, D), dt),
            pltpu.VMEM((D, F), dt),
            pltpu.VMEM((D, F), dt),
            pltpu.VMEM((F, D), dt),
            pltpu.VMEM((B, D), dt),
            pltpu.VMEM((D,), dt),
            pltpu.VMEM((2 * B, D), f32),
            pltpu.VMEM((2 * B, D), f32),
            pltpu.VMEM((2 * B, HD), f32),
            pltpu.VMEM((_RING, B * HD + _WIN), f32),
            pltpu.VMEM((_RING, B * HD + 2 * _WIN), f32),
            pltpu.VMEM((B * _RING, HD), f32),
            pltpu.VMEM((_RING, Sk), f32),
            pltpu.VMEM((_RING, Sk), f32),
            pltpu.VMEM((_RING, 1), f32),
            pltpu.VMEM((_RING, _WIN), f32),
            pltpu.VMEM((B * _RING, D), f32),
            pltpu.VMEM((2 * B, F), f32),
            pltpu.VMEM((2 * B, D), f32),
            pltpu.SemaphoreType.DMA((_NB,)),
            pltpu.SemaphoreType.DMA((_NB,)),
            pltpu.SemaphoreType.DMA((_PARTS,)),
            pltpu.SemaphoreType.DMA((7,)),
        ],
        compiler_params=pltpu.CompilerParams(
            vmem_limit_bytes=96 * 1024 * 1024, disable_bounds_checks=True
        ),
    )(A_x.reshape(B, D), kt, vt, A_wq, A_wo, B_w_r, B_w_gate, B_w_up, B_w_down)
    return out.reshape(B, Sq, D)
```

```python
import functools

import jax
import jax.numpy as jnp
import jax.experimental.pallas as pl
import jax.experimental.pallas.tpu as pltpu

_EPS = 1e-5
_NB = 3
_WIN = 512
_QTR = 128
_GC = 1024
_VISITS = 64
_STEPS = 16
_LEAD = 16
_PACE = (3, 2, 2, 2, 4)
_K_START = 1
_V_START = 37
_K_PAD = 336
_V_PAD = 544
_RING = 8
_SLAB = 32
_PARTS = 6
_EARLY = 4


def _layernorm(x):
    m = jnp.mean(x, axis=-1, keepdims=True)
    d = x - m
    v = jnp.mean(d * d, axis=-1, keepdims=True)
    return d / jnp.sqrt(v + _EPS)


def _dot(a, b):
    return jnp.dot(a, b, preferred_element_type=jnp.float32)


def _dot_nt(a, b):
    return jax.lax.dot_general(
        a, b, (((1,), (1,)), ((), ())), preferred_element_type=jnp.float32
    )


def _wait_all(buf, sem):
    pltpu.make_async_copy(buf, buf, sem).wait()


def _ds(start, size):
    return pl.ds(start if isinstance(start, int) else pl.multiple_of(start, size), size)


def _loop(lo, hi, fn):
    jax.lax.fori_loop(lo, hi, lambda i, carry: fn(i), None)


def _body(
    x_hbm, kt_hbm, vt_hbm, wq_hbm, wo_hbm, wr_hbm, wg_hbm, wu_hbm, wd_hbm,
    out_ref,
    kbuf, vbuf, vend, wqbuf, wobuf, wgbuf, wubuf, wdbuf, xbuf, wrbuf,
    x_scr, n_scr, t_scr, q_scr, o_scr, ob_scr, s_scr, p_scr, l_scr, pv_scr, a_scr, g_scr, y_scr,
    ksem, vsem, dsem, sem,
    *, B, H, Dh, Sk, D, F,
):
    HD = H * Dh
    last = B * HD // _WIN
    k_first = _WIN - _K_PAD
    v_end = _V_PAD - _WIN
    half = _STEPS // 2
    scale = Dh ** -0.5
    f32, bf16 = jnp.float32, jnp.bfloat16
    X, WR, WQ, VE, WO, G0, G1, U0, U1 = (sem.at[i] for i in range(9))

    def copy(src, dst, dma_sem, queue):
        pltpu.make_async_copy(src, dst, dma_sem).start(priority=queue)

    def window_piece(hbm, buf, dma_sem, pad, p, g, second, quarter, n, queue):
        slot = jax.lax.rem(p, _NB)
        cols = _ds((g & 7) * _GC, _GC)
        at = second * (_QTR // 2) + (g >> 3) * 8
        row = p * _WIN - pad + at
        copy(
            hbm.at[pl.ds((row >> 7) + quarter, n), _ds(row & (_QTR - 1), 8), cols],
            buf.at[slot, pl.ds(quarter, n), _ds(at, 8), cols],
            dma_sem.at[slot],
            queue,
        )

    def cache_piece(hbm, buf, dma_sem, row, buf_row):
        def piece(g, queue):
            r, cols = (g >> 2) * 8, _ds((g & 3) * 2 * _GC, 2 * _GC)
            src, dst = row + r, buf_row + r
            copy(
                hbm.at[src >> 7, _ds(src & (_QTR - 1), 8), cols],
                buf.at[dst >> 7, _ds(dst & (_QTR - 1), 8), cols],
                dma_sem,
                queue,
            )

        return piece

    def wq_piece(g, queue):
        row = g * 171 >> 9
        where = (_ds(row * 8, 8), _ds((g - 3 * row) * 2 * _GC, 2 * _GC))
        copy(wq_hbm.at[where], wqbuf.at[where], WQ, queue)

    def row_piece(hbm, buf, dma_sem, rows, cols=slice(None)):
        def piece(g, queue):
            where = (_ds(g * rows, rows), cols)
            copy(hbm.at[where], buf.at[where], dma_sem, queue)

        return piece

    def down_piece(g, queue):
        rows = _ds(g * _SLAB, _SLAB)
        copy(wd_hbm.at[rows], wdbuf.at[rows], dsem.at[g >> 3], queue)

    end_slot = last % _NB
    units = F // _PARTS
    early, late = pl.ds(0, _EARLY * units), pl.ds(_EARLY * units, F - _EARLY * units)
    head = (
        ([wq_piece], D // 8 * HD // (2 * _GC), 16),
        ([cache_piece(kt_hbm, kbuf.at[0], ksem.at[0], 0, _K_PAD)], k_first // 2, 8),
    )
    tail = (
        ([cache_piece(kt_hbm, kbuf.at[end_slot], ksem.at[end_slot], B * HD - _K_PAD, 0)],
         _K_PAD // 2, 8),
        ([cache_piece(vt_hbm, vbuf.at[end_slot], vsem.at[end_slot], B * HD - _V_PAD, 0)],
         _WIN // 2, 16),
        ([cache_piece(vt_hbm, vend, VE, B * HD - v_end, 0)], v_end // 2, 4),
        ([row_piece(wo_hbm, wobuf, WO, _SLAB)], HD // _SLAB, 8),
        ([row_piece(wg_hbm, wgbuf, G0, 16, early), row_piece(wu_hbm, wubuf, U0, 16, early)],
         D // 8, 4),
        ([row_piece(wg_hbm, wgbuf, G1, 32, late), row_piece(wu_hbm, wubuf, U1, 32, late)],
         D // 16, 4),
        ([down_piece], F // _SLAB, 1),
    )
    u_lo = -sum(n for _, n, _ in head) // 8
    u_mid = (last - 1) * _VISITS
    u_hi = u_mid + sum(n for _, n, _ in tail) // 8

    def other_visits(at, parts, lo, hi):
        for fns, n, runs in parts:
            assert n % (runs * len(fns)) == 0

            def pair(i, fns=fns, n=n, runs=runs):
                for c in range(2):
                    k = i if len(fns) == 2 else 2 * i + c
                    turn = k >> (runs.bit_length() - 1)
                    fns[c % len(fns)]((k & (runs - 1)) * (n // len(fns) // runs) + turn, c)

            _loop(4 * jnp.clip(lo - at, 0, n // 8), 4 * jnp.clip(hi - at, 0, n // 8), pair)
            at += n // 8

    def window_visits(u):
        p = (u >> 6) + 1
        k_piece = functools.partial(window_piece, kt_hbm, kbuf, ksem, _K_PAD, p)
        v_piece = functools.partial(window_piece, vt_hbm, vbuf, vsem, _V_PAD, p)

        def visit(i):
            quarter = (i & 1) * 2
            for d in range(2):
                gk = (u + (i & 2) + d + _K_START) & (_VISITS - 1)
                gv = (u + (i & 2) + d + _V_START) & (_VISITS - 1)
                cut = (p == 1) & (quarter == 0) & (gv < v_end)
                k_piece(gk, 0, quarter, 2, 0)
                pl.when(cut)(lambda: v_piece(gv, 0, 1, 1, 1))
                pl.when(jnp.logical_not(cut))(lambda: v_piece(gv, 0, quarter, 2, 1))
                k_piece(gk, 1, quarter, 2, 0)
                v_piece(gv, 1, quarter, 2, 1)

        _loop(0, 4, visit)

    w_last = last * _STEPS

    def issued(w, clip=jnp.clip):
        u = 4 * clip(w, u_lo, w_last - _STEPS)
        for i, pace in enumerate(_PACE):
            u += pace * clip(w - w_last + _STEPS - i * half, 0, half)
        return clip(u + _LEAD, u_lo + 1, u_hi)

    def issue(w):
        lo, hi = issued(w - 1), issued(w)
        pl.when(lo < 0)(lambda: other_visits(u_lo, head, lo, hi))
        pl.when(jnp.logical_and(lo >= 0, lo < u_mid))(lambda: window_visits(lo))
        pl.when(jnp.logical_and(lo >= u_mid, lo < hi))(lambda: other_visits(u_mid, tail, lo, hi))

    def owned(first_row, width):
        span = _RING * Dh
        r = jax.lax.broadcasted_iota(jnp.int32, (_RING, width), 1) + first_row
        r = jnp.where(r >= span, r - span, r)
        lo = jax.lax.broadcasted_iota(jnp.int32, (_RING, width), 0) * Dh
        return (r >= lo) & (r < lo + Dh)

    def prepare():
        copy(x_hbm, xbuf, X, 0)
        copy(wr_hbm, wrbuf, WR, 1)

        def clear(i):
            kbuf[0, i >> 3, _ds((i & 7) * 16, 16), :] = jnp.zeros((16, Sk), kbuf.dtype)

        def clear_cols(i):
            vbuf[1, 0, pl.ds(0, v_end), _ds(i * _GC, _GC)] = jnp.zeros((v_end, _GC), vbuf.dtype)
            s_scr[:, _ds(i * _GC, _GC)] = jnp.zeros((_RING, _GC), f32)
            p_scr[:, _ds(i * _GC, _GC)] = jnp.zeros((_RING, _GC), f32)

        _loop(0, _K_PAD // 16, clear)
        _loop(0, half, clear_cols)
        l_scr[...] = jnp.ones_like(l_scr)
        q_scr[:, pl.ds(0, _WIN)] = jnp.zeros((_RING, _WIN), f32)
        q_scr[:, pl.ds(B * HD, _WIN)] = jnp.zeros((_RING, _WIN), f32)

    def project(i):
        @pl.when(i == 0)
        def _():
            _wait_all(xbuf, X)
            x = xbuf[...].astype(f32)
            x_scr[...] = jnp.concatenate([x, x], axis=0)
            n_scr[...] = _layernorm(x_scr[...])
            _wait_all(wqbuf, WQ)

        def part(k):
            cols = _ds((4 * i + k) * 512, 512)
            t_scr[:, cols] = _dot(n_scr[...].astype(bf16), wqbuf[:, cols])

        _loop(0, 4, part)

    def lay_out_queries():
        span = _RING * Dh
        base, shift = _K_PAD // 128 * 128, _K_PAD % 128
        mine = owned(0, span)
        keep = jax.lax.broadcasted_iota(jnp.int32, (_RING, 128), 1) < shift

        def group(i):
            b = jax.lax.div(i, HD // span)
            q = t_scr[pl.ds(b, 1), _ds((i - b * (HD // span)) * span, span)]
            q = jnp.concatenate([jnp.where(mine, q, 0.0), jnp.zeros((_RING, 128), f32)], axis=1)
            q = pltpu.roll(q, shift, 1)
            at = pl.multiple_of(base + i * span, 128)
            q_scr[:, pl.ds(at, 128)] = jnp.where(keep, q_scr[:, pl.ds(at, 128)], q[:, :128])
            q_scr[:, pl.ds(at + 128, span)] = q[:, 128:]

        _loop(0, B * HD // span, group)

    def await_rows(buf, dma_sem, p, lo, hi):
        first, end = -(-lo // _QTR), hi // _QTR
        window, dma_sem = buf.at[p % _NB], dma_sem.at[p % _NB]
        if lo % _QTR:
            _wait_all(window.at[first - 1, pl.ds(lo % _QTR, _QTR - lo % _QTR)], dma_sem)
        _wait_all(window.at[pl.ds(first, end - first)], dma_sem)
        if hi % _QTR:
            _wait_all(window.at[end, pl.ds(0, hi % _QTR)], dma_sem)

    def score(p, j):
        slot = jax.lax.rem(p, _NB)

        @pl.when(j == 0)
        def _():
            pl.when(p == 0)(lambda: await_rows(kbuf, ksem, 0, _K_PAD, _WIN))
            pl.when(p == last)(lambda: await_rows(kbuf, ksem, last, 0, _K_PAD))
            pl.when((p > 0) & (p < last))(lambda: _wait_all(kbuf.at[slot], ksem.at[slot]))

        cols = _ds(j * _GC, _GC)
        q = q_scr[:, _ds(p * _WIN, _WIN)].astype(bf16)
        s_scr[:, cols] += _dot(q, kbuf[slot, :, :, cols].reshape(_WIN, _GC))

    def softmax(p):
        end = (p + 1) * _WIN - _K_PAD
        done_hi = jax.lax.div(jnp.minimum(end, B * HD), Dh)
        done_lo = jax.lax.div(jnp.maximum(end - _WIN, 0), Dh)
        ring_row = jax.lax.broadcasted_iota(jnp.int32, (_RING, 1), 0)
        done = (ring_row - done_lo) & (_RING - 1) < done_hi - done_lo
        raw = s_scr[...]
        s = raw * scale
        e = jnp.exp(s - jnp.max(s, axis=-1, keepdims=True))
        p_scr[...] = jnp.where(done, e, p_scr[...])
        l_scr[...] = jnp.where(done, jnp.sum(e, axis=-1, keepdims=True), l_scr[...])
        s_scr[...] = jnp.where(done, 0.0, raw)

    def mix(p, j):
        slot = jax.lax.rem(p, _NB)

        @pl.when(j == 0)
        def _():
            pl.when(p == 1)(lambda: await_rows(vbuf, vsem, 1, v_end, _WIN))
            pl.when(p > 1)(lambda: _wait_all(vbuf.at[slot], vsem.at[slot]))
            pv_scr[...] = jnp.zeros_like(pv_scr)

        cols = _ds(j * _GC, _GC)
        v = vbuf[slot, :, :, cols].reshape(_WIN, _GC)
        pv_scr[...] += _dot_nt(p_scr[:, cols].astype(bf16), v)

        @pl.when(j == half - 1)
        def _():
            span = _RING * Dh
            mine = owned(jax.lax.rem(p * _WIN - _V_PAD + span, span), _WIN)
            o_scr[:, _ds(p * _WIN, _WIN)] = jnp.where(mine, pv_scr[...] / l_scr[...], 0.0)

    def attend(w):
        p, j = w >> 4, w & (_STEPS - 1)
        pl.when(j < half)(lambda: score(p, j))
        pl.when(j == half)(lambda: softmax(p))
        pl.when(jnp.logical_and(j >= half, p > 0))(lambda: mix(p, j - half))

    def lay_out_values(lo, hi):
        def group(i):
            b, c = i >> 2, (i & 3) * (HD // 4)
            o = o_scr[:, pl.ds(pl.multiple_of(_WIN + i * (HD // 4), 128), HD // 4 + 128)]
            ob_scr[_ds(b * _RING, _RING), _ds(c, HD // 4)] = o[:, v_end:v_end + HD // 4]

        _loop(lo, hi, group)

    def finish_values():
        _wait_all(vend, VE)
        pv = _dot_nt(p_scr[...].astype(bf16), vend[0])
        mine = owned(_RING * Dh - v_end, v_end)
        o_scr[:, pl.ds((last + 1) * _WIN, 128)] = jnp.zeros((_RING, 128), f32)
        o_scr[:, pl.ds((last + 1) * _WIN, v_end)] = jnp.where(mine, pv / l_scr[...], 0.0)
        lay_out_values(4 * B - 2, 4 * B)
        a_scr[...] = jnp.zeros_like(a_scr)

    def merge(i):
        pl.when(i == 0)(lambda: _wait_all(wobuf, WO))
        rows = _ds(i * (HD // _PARTS), HD // _PARTS)
        a_scr[...] += _dot(ob_scr[:, rows].astype(bf16), wobuf[rows, :])

    w_end = (last + 1) * _STEPS

    def step(w):
        issue(w)
        pl.when(w == -8)(prepare)
        pl.when(jnp.logical_and(w >= -3, w < 0))(lambda: project(w + 3))
        pl.when(w == -1)(lay_out_queries)
        pl.when(jnp.logical_and(w >= 0, w < w_end))(lambda: attend(w))
        pl.when(w == w_last - 2 * _STEPS)(lambda: lay_out_values(0, 4 * B - 2))
        pl.when(w == w_end)(finish_values)
        pl.when(w >= w_end)(lambda: merge(w - w_end))

    u_caches = u_mid + (_K_PAD + _V_PAD) // 16
    for w, u in ((-3, -k_first // 16), (w_last, u_caches - _V_PAD // 16), (w_last + half, u_caches),
                 (w_end, u_caches + HD // _SLAB // 8), (w_end + _PARTS - 1, u_hi)):
        assert issued(w, lambda v, lo, hi: min(max(v, lo), hi)) >= u and _LEAD % 4 == 0
    for k in range(8):
        wq_piece(k * (head[0][1] // head[0][2]), k % 2)
    w_lo = (u_lo + 1 - _LEAD) // 4 + 1
    _loop(0, w_end + _PARTS - w_lo, lambda i: step(i + w_lo))

    attn = jnp.sum(a_scr[...].reshape(B, _RING, D), axis=1)
    h = x_scr[...] + jnp.concatenate([attn, attn], axis=0)
    hn = _layernorm(h)
    n_scr[...] = hn
    _wait_all(wrbuf, WR)
    r = jnp.sum(hn * wrbuf[...].astype(f32).reshape(1, D), axis=-1, keepdims=True)
    route = jax.nn.sigmoid(r)

    def activate(f):
        cols = _ds(f * units, units)
        hb = n_scr[...].astype(bf16)
        gate = _dot(hb, wgbuf[:, cols])
        g_scr[:, cols] = gate * jax.nn.sigmoid(gate) * _dot(hb, wubuf[:, cols])

    def reduce(f):
        rows = _ds(f * units, units)
        _wait_all(wdbuf.at[rows], dsem.at[f])
        y_scr[...] += _dot(g_scr[:, rows].astype(bf16), wdbuf[rows, :])

    def feed_forward(i):
        for k, (cols, gate_sem, up_sem) in enumerate(((early, G0, U0), (late, G1, U1))):
            @pl.when(i == k)
            def _():
                _wait_all(wgbuf.at[:, cols], gate_sem)
                _wait_all(wubuf.at[:, cols], up_sem)

        _loop(i * _EARLY, _EARLY + i * (_PARTS - _EARLY), activate)

    _loop(0, 2, feed_forward)
    y_scr[...] = jnp.zeros_like(y_scr)
    _loop(0, _PARTS, reduce)
    y = y_scr[...] * route
    out = h + (hn + (hn * 0.0 + y))
    out_ref[...] = out[:B].astype(out_ref.dtype)


@jax.jit
def pallas_sequential_preLN__mha_block_cached__moe_arch_mod__decode_kernel(
    A_x: jax.Array,
    A_k_cache: jax.Array,
    A_v_cache: jax.Array,
    A_wq: jax.Array,
    A_wo: jax.Array,
    B_x: jax.Array,
    B_w_r: jax.Array,
    B_w_gate: jax.Array,
    B_w_up: jax.Array,
    B_w_down: jax.Array,
):
    del B_x
    B, Sq, D = A_x.shape
    _, H, Sk, Dh = A_k_cache.shape
    F = B_w_gate.shape[1]
    HD = H * Dh
    assert (B, Sq, D, H, Sk, Dh, F) == (4, 1, 640, 32, 8 * _GC, 192, 1536)
    dt = A_k_cache.dtype
    f32 = jnp.float32

    kt = jnp.swapaxes(A_k_cache, 2, 3).reshape(B * HD // _QTR, _QTR, Sk)
    vt = jnp.swapaxes(A_v_cache, 2, 3).reshape(B * HD // _QTR, _QTR, Sk)

    out = pl.pallas_call(
        functools.partial(_body, B=B, H=H, Dh=Dh, Sk=Sk, D=D, F=F),
        in_specs=[pl.BlockSpec(memory_space=pl.ANY)] * 9,
        out_specs=pl.BlockSpec(memory_space=pltpu.VMEM),
        out_shape=jax.ShapeDtypeStruct((B, D), A_x.dtype),
        scratch_shapes=[
            pltpu.VMEM((_NB, _WIN // _QTR, _QTR, Sk), dt),
            pltpu.VMEM((_NB, _WIN // _QTR, _QTR, Sk), dt),
            pltpu.VMEM((1, _V_PAD - _WIN, Sk), dt),
            pltpu.VMEM((D, HD), dt),
            pltpu.VMEM((HD, D), dt),
            pltpu.VMEM((D, F), dt),
            pltpu.VMEM((D, F), dt),
            pltpu.VMEM((F, D), dt),
            pltpu.VMEM((B, D), dt),
            pltpu.VMEM((D,), dt),
            pltpu.VMEM((2 * B, D), f32),
            pltpu.VMEM((2 * B, D), f32),
            pltpu.VMEM((2 * B, HD), f32),
            pltpu.VMEM((_RING, B * HD + _WIN), f32),
            pltpu.VMEM((_RING, B * HD + 2 * _WIN), f32),
            pltpu.VMEM((B * _RING, HD), f32),
            pltpu.VMEM((_RING, Sk), f32),
            pltpu.VMEM((_RING, Sk), f32),
            pltpu.VMEM((_RING, 1), f32),
            pltpu.VMEM((_RING, _WIN), f32),
            pltpu.VMEM((B * _RING, D), f32),
            pltpu.VMEM((2 * B, F), f32),
            pltpu.VMEM((2 * B, D), f32),
            pltpu.SemaphoreType.DMA((_NB,)),
            pltpu.SemaphoreType.DMA((_NB,)),
            pltpu.SemaphoreType.DMA((_PARTS,)),
            pltpu.SemaphoreType.DMA((9,)),
        ],
        compiler_params=pltpu.CompilerParams(
            vmem_limit_bytes=96 * 1024 * 1024, disable_bounds_checks=True
        ),
    )(A_x.reshape(B, D), kt, vt, A_wq, A_wo, B_w_r, B_w_gate, B_w_up, B_w_down)
    return out.reshape(B, Sq, D)
```
